```python
import os as _os
_os.environ.setdefault("JAX_PLATFORMS", "cpu")
import jax
import jax.numpy as jnp

def _softmax(x, axis=-1):
    return jax.nn.softmax(x, axis=axis)
def _gelu(x):
    return jax.nn.gelu(x, approximate=True)
def _silu(x):
    return jax.nn.silu(x)
def _sigmoid(x):
    return jax.nn.sigmoid(x)
def _layernorm(x, axis=-1, eps=1e-5):
    m = jnp.mean(x, axis=axis, keepdims=True)
    v = jnp.var(x, axis=axis, keepdims=True)
    return (x - m) / jnp.sqrt(v + eps)
def _scatter_add(tgt, idx, src, axis=0):
    return tgt.at[idx].add(src)
def _segment_sum(src, seg, n):
    return jax.ops.segment_sum(src, seg, n)
class _Rng:
    def __init__(self, key):
        self._k = key
    def _next(self):
        self._k, sub = jax.random.split(self._k)
        return sub
    def normal(self, shape):
        return jax.random.normal(self._next(), shape, dtype=jnp.bfloat16)
    def randint(self, lo, hi, shape):
        return jax.random.randint(self._next(), shape, lo, hi, dtype=jnp.int32)
    def uniform(self, shape, lo=0.0, hi=1.0):
        return jax.random.uniform(self._next(), shape, jnp.bfloat16, lo, hi)
    def permutation(self, n):
        return jax.random.permutation(self._next(), n)


kernel_name = 'concat_heads__sliding_block__grouped_kv_mqa__prompt'

def setup_inputs():
    _rng = _Rng(jax.random.key(int.from_bytes(__import__("os").urandom(4), "little")))
    _w = (lambda a: (lambda t: t.astype(jnp.bfloat16) if jnp.issubdtype(t.dtype, jnp.floating) else t)(jnp.asarray(a)))
    def _A_setup():
        B, S, D = 1, 2048, 576
        return {
            "x": _w((lambda *s: _rng.normal(s) * 0.2)(B, S, D)),
            "wqkv": _w((lambda *s: _rng.normal(s) * 0.2)(D, 3 * D)),
            "wo": _w((lambda *s: _rng.normal(s) * 0.05)(D, D)),
        }
    _A_in = _A_setup()

    def _B_setup():
        B, S, D, H = 1, 2048, 576, 32
        Dh = D // H
        return {
            "x": _w((lambda *s: _rng.normal(s) * 0.05)(B, S, D)),
            "wq": _w((lambda *s: _rng.normal(s) * 1.6)(D, H * Dh)),
            "wk": _w((lambda *s: _rng.normal(s) * 1.6)(D, Dh)),
            "wv": _w((lambda *s: _rng.normal(s) * 0.1)(D, Dh)),
            "wo": _w((lambda *s: _rng.normal(s) * 0.1)(H * Dh, D)),
        }
    _B_in = _B_setup()

    return {
        "A_x": _A_in["x"],
        "A_wqkv": _A_in["wqkv"],
        "A_wo": _A_in["wo"],
        "B_x": _B_in["x"],
        "B_wq": _B_in["wq"],
        "B_wk": _B_in["wk"],
        "B_wv": _B_in["wv"],
        "B_wo": _B_in["wo"],
    }

def reference(A_x, A_wqkv, A_wo, B_x, B_wq, B_wk, B_wv, B_wo):
    def _A_ref(x, wqkv, wo):
        B, S, D = x.shape
        H = 32; Dh = D // H; W = 256
        qkv = (lambda x, *d: x.transpose(*d))((x @ wqkv).reshape(B, S, 3, H, Dh), 2, 0, 3, 1, 4)
        q, k, v = qkv[0], qkv[1], qkv[2]
        scores = jnp.einsum("bhqd,bhkd->bhqk", q, k) * (Dh ** -0.5)
        idx = jnp.arange(S)
        mask = (idx[:, None] - idx[None, :] >= 0) & (idx[:, None] - idx[None, :] < W)
        scores = jnp.where(mask[None, None], scores, -1e9)
        p = _softmax(scores, axis=-1)
        o = jnp.einsum("bhqk,bhkd->bhqd", p, v)
        return (lambda x, *d: x.transpose(*d))(o, 0, 2, 1, 3).reshape(B, S, D) @ wo

    def _B_ref(x, wq, wk, wv, wo):
        B, S, D = x.shape
        H = 32
        Dh = D // H
        q = (lambda x, *d: x.transpose(*d))((x @ wq).reshape(B, S, H, Dh), 0, 2, 1, 3)
        k = x @ wk
        v = x @ wv
        scores = jnp.einsum("bhqd,bkd->bhqk", q, k) * (Dh ** -0.5)
        p = _softmax(scores, axis=-1)
        o = jnp.einsum("bhqk,bkd->bhqd", p, v)
        return (lambda x, *d: x.transpose(*d))(o, 0, 2, 1, 3).reshape(B, S, H * Dh) @ wo

    a = _A_ref(A_x, A_wqkv, A_wo)
    b = _B_ref(B_x, B_wq, B_wk, B_wv, B_wo)
    return jnp.concatenate([a, b], axis=-1)
```

```python
import functools
import jax
import jax.numpy as jnp
import numpy as np
from jax import lax
from jax.experimental import pallas as pl
from jax.experimental.pallas import tpu as pltpu

S = 2048
D = 576
H = 32
DH = 18
NG = 5
TQ = 512
NEG = -1e30
QSCALE = float(DH ** -0.5 * np.log2(np.e))
F32 = jnp.float32
BF16 = jnp.bfloat16


def _pad_group_rows(wt):
    n = wt.shape[1]
    parts = []
    for g in range(NG):
        lo = 126 * g
        hi = min(lo + 126, D)
        parts.append(wt[lo:hi])
        parts.append(jnp.zeros((128 - (hi - lo), n), wt.dtype))
    return jnp.concatenate(parts, axis=0)


def _assemble(o, row8):
    def sel(k, a, b):
        return jnp.where(row8 < k, a, b)
    return jnp.concatenate([
        o[0][0:8], o[0][8:16], sel(2, o[0][16:24], o[1][0:8]),
        o[1][8:16], sel(4, o[1][16:24], o[2][0:8]),
        o[2][8:16], sel(6, o[2][16:24], o[3][0:8]),
        o[3][8:16], o[3][16:24]], axis=0)


def _lrow(jj):
    return 23 if jj < 3 else 0


def kernel_body(axT_h, awqkv_h, awo_h, bxT_h, bwq_h, bwkT_h, bwvT_h, bwo_h,
                out_h,
                xa_s, xb_s, wqkv_s, wq_s, wo_s, wkv_s,
                wqT_s, wkT_s, wvT_s, woT_s, qT_s, kvar_s, vTb_s, sB_s, mB_s, oB_s,
                kA_s, vTa_s, sA_s, mA_s, oA_s, out_s, sems, osems):
    NC = S // TQ

    def cp(src, dst, i):
        return pltpu.make_async_copy(src, dst, sems.at[i])

    def xcopy(h, s, c, i):
        return cp(h.at[:, pl.ds(c * TQ, TQ)], s.at[:, pl.ds(c * TQ, TQ)], i)

    c_wq = cp(bwq_h, wq_s, 0)
    c_wk = cp(bwkT_h, wkv_s.at[0], 1)
    c_wv = cp(bwvT_h, wkv_s.at[1], 2)
    c_xb = [xcopy(bxT_h, xb_s, c, 3 + c) for c in range(NC)]
    c_wob = cp(bwo_h, wo_s.at[1], 7)
    c_wqkv = cp(awqkv_h, wqkv_s, 8)
    c_xa = cp(axT_h, xa_s, 9)
    c_woa = cp(awo_h, wo_s.at[0], 10)

    c_wq.start()
    c_wk.start()
    c_wv.start()
    c_xb[0].start()

    lane = lax.broadcasted_iota(jnp.int32, (1, 128), 1)

    c_wk.wait()
    c_wv.wait()
    wkT = wkv_s[0].astype(F32)
    wvT = wkv_s[1].astype(F32)
    wkvT = jnp.concatenate([wkT] * 7 + [jnp.zeros((2, D), F32), wvT, jnp.zeros((14, D), F32)],
                           axis=0).astype(BF16)
    c_wq.wait()
    wqT_s[...] = _pad_group_rows(wq_s[...].astype(F32).T).astype(BF16)
    row24 = lax.broadcasted_iota(jnp.int32, (24, TQ), 0)
    for c in range(NC):
        c_xb[c].wait()
        if c + 1 < NC:
            c_xb[c + 1].start()
        else:
            c_wob.start()
            c_wqkv.start()
            c_xa.start()
            c_woa.start()
        xT = xb_s[:, pl.ds(c * TQ, TQ)]
        qT = jnp.dot(wqT_s[...], xT, preferred_element_type=F32) * QSCALE
        qT_s[:, pl.ds(c * TQ, TQ)] = qT.astype(BF16)
        kvT = jnp.dot(wkvT, xT, preferred_element_type=F32)
        kr = kvT[0:128].T
        for j in range(7):
            kvar_s[j, pl.ds(c * TQ, TQ), :] = jnp.where(
                (lane >= DH * j) & (lane < DH * j + DH), kr, 0.0).astype(BF16)
        vT = kvT[128:152].astype(BF16).astype(F32)
        for jj in range(4):
            off = 2 * jj
            if off:
                vv = jnp.concatenate([jnp.zeros((off, TQ), F32), vT[0:24 - off]], axis=0)
            else:
                vv = vT
            vTb_s[jj, :, pl.ds(c * TQ, TQ)] = jnp.where(row24 == _lrow(jj), 1.0, vv)

    NCH = S // 128
    row8 = lax.broadcasted_iota(jnp.int32, (8, TQ), 0)

    def b_qk_chunk(it, c, slot, m):
        qt = it // H
        h = it % H
        g = h // 7
        j = h % 7
        w = qT_s[pl.ds(pl.multiple_of(g * 128, 128), 128), pl.ds(pl.multiple_of(qt * TQ, TQ), TQ)]
        s = jnp.dot(kvar_s[j, pl.ds(c * 128, 128), :], w, preferred_element_type=F32)
        sB_s[slot, pl.ds(c * 128, 128), :] = s
        mm = jnp.max(s.reshape(16, 8, TQ), axis=0)
        return mm if m is None else jnp.maximum(m, mm)

    def b_fin_m(m8, slot):
        mB_s[slot] = jnp.broadcast_to(jnp.max(m8, axis=0, keepdims=True), (8, TQ))

    def b_pv_chunk(c, slot, jj, m, acc):
        p = jnp.exp2(sB_s[slot, pl.ds(c * 128, 128), :] - m).astype(BF16)
        o = jnp.dot(vTb_s[jj, :, pl.ds(c * 128, 128)], p, preferred_element_type=F32)
        return o if acc is None else acc + o

    m = None
    for c in range(NCH):
        m = b_qk_chunk(0, c, 0, m)
    b_fin_m(m, 0)
    NIT = (S // TQ) * H

    def b_body(i, carry):
        outs = []
        for jj in range(4):
            it = i * 4 + jj
            slot = jj % 2
            itn = jnp.minimum(it + 1, NIT - 1)
            mcur = mB_s[slot][0:1, :]
            mn = None
            acc = None
            for c in range(NCH):
                mn = b_qk_chunk(itn, c, 1 - slot, mn)
                acc = b_pv_chunk(c, slot, jj, mcur, acc)
            b_fin_m(mn, 1 - slot)
            lr = _lrow(jj)
            outs.append(acc * (1.0 / acc[lr:lr + 1, :]))
        qt = i // 8
        u = i % 8
        oB_s[pl.ds(pl.multiple_of(u * 72, 8), 72), pl.ds(pl.multiple_of(qt * TQ, TQ), TQ)] = _assemble(outs, row8)
        return carry

    lax.fori_loop(0, NIT // 4, b_body, 0)

    c_wob.wait()
    c_wqkv.wait()
    c_xa.wait()
    c_woa.wait()
    wT = wqkv_s[...].astype(F32).T
    wqT_s[...] = _pad_group_rows(wT[0:D]).astype(BF16)
    wkT_s[...] = _pad_group_rows(wT[D:2 * D]).astype(BF16)
    wvT_s[...] = wT[2 * D:3 * D].astype(BF16)
    woT_s[0] = wo_s[0].astype(F32).T.astype(BF16)
    woT_s[1] = wo_s[1].astype(F32).T.astype(BF16)
    for g in range(NG):
        kA_s[g, 0:256, :] = jnp.broadcast_to(jnp.where(lane == 127, 1.0, 0.0), (256, 128)).astype(BF16)
    vTa_s[:, 0:256] = jnp.zeros((D, 256), F32)
    for c in range(NC):
        xT = xa_s[:, pl.ds(c * TQ, TQ)]
        qT = jnp.dot(wqT_s[...], xT, preferred_element_type=F32) * QSCALE
        qT_s[:, pl.ds(c * TQ, TQ)] = qT.astype(BF16)
        kT = jnp.dot(wkT_s[...], xT, preferred_element_type=F32)
        for g in range(NG):
            kA_s[g, pl.ds(256 + c * TQ, TQ), :] = kT[128 * g:128 * (g + 1)].T.astype(BF16)
        vT = jnp.dot(wvT_s[...], xT, preferred_element_type=F32)
        vTa_s[:, pl.ds(256 + c * TQ, TQ)] = vT.astype(BF16).astype(F32)

    r128 = lax.broadcasted_iota(jnp.int32, (128, 128), 0)
    l128 = lax.broadcasted_iota(jnp.int32, (128, 128), 1)
    r16 = lax.broadcasted_iota(jnp.int32, (16, 128), 0)
    r24 = lax.broadcasted_iota(jnp.int32, (24, 384), 0)
    row8a = lax.broadcasted_iota(jnp.int32, (8, 128), 0)

    def a_qk_head(qt, h, slot, hh):
        g, j = h // 7, h % 7
        q0 = pl.multiple_of(qt * 128, 128)
        lo, hi = DH * j, DH * j + DH
        blocks = []
        for b in range(8):
            r0 = 16 * b
            if r0 + 16 <= lo or r0 >= hi:
                blk = None
            else:
                blk = qT_s[pl.ds(128 * g + r0, 16), pl.ds(q0, 128)]
                if not (r0 >= lo and r0 + 16 <= hi):
                    blk = jnp.where((r16 + r0 >= lo) & (r16 + r0 < hi), blk, jnp.zeros_like(blk))
            if b == 7:
                neg = jnp.where(r16 == 15, NEG, 0.0).astype(BF16)
                blk = neg if blk is None else jnp.where(r16 == 15, neg, blk)
            if blk is None:
                blk = jnp.zeros((16, 128), BF16)
            blocks.append(blk)
        w = jnp.concatenate(blocks, axis=0)
        s = jnp.dot(kA_s[g, pl.ds(q0, 384), :], w, preferred_element_type=F32)
        s0 = jnp.where(r128 > l128, s[0:128], NEG)
        s1 = s[128:256]
        s2 = jnp.where(r128 <= l128, s[256:384], NEG)
        sA_s[slot, hh, 0:128, :] = s0
        sA_s[slot, hh, 128:256, :] = s1
        sA_s[slot, hh, 256:384, :] = s2
        mm = jnp.maximum(jnp.maximum(s0, s1), s2)
        mm = jnp.max(mm.reshape(16, 8, 128), axis=0)
        mm = jnp.max(mm, axis=0, keepdims=True)
        mA_s[slot, hh] = jnp.broadcast_to(mm, (8, 128))

    def a_pv_head(qt, h, slot, hh):
        q0 = pl.multiple_of(qt * 128, 128)
        r0 = (DH * h) // 8 * 8
        lr = _lrow(h % 4)
        m = mA_s[slot, hh][0:1, :]
        p = jnp.exp2(sA_s[slot, hh] - m).astype(BF16)
        v = jnp.where(r24 == lr, 1.0, vTa_s[r0:r0 + 24, pl.ds(q0, 384)])
        o = jnp.dot(v, p, preferred_element_type=F32)
        return o * (1.0 / o[lr:lr + 1, :])

    NQT = S // 128
    for hh in range(4):
        a_qk_head(0, hh, 0, hh)

    def a_body(qt, carry):
        for s in range(8):
            slot = s % 2
            if s < 7:
                nqt, nh0 = qt, (s + 1) * 4
            else:
                nqt, nh0 = jnp.minimum(qt + 1, NQT - 1), 0
            for hh in range(4):
                a_qk_head(nqt, nh0 + hh, 1 - slot, hh)
            outs = [a_pv_head(qt, s * 4 + hh, slot, hh) for hh in range(4)]
            oA_s[pl.ds(72 * s, 72), pl.ds(pl.multiple_of((qt % 4) * 128, 128), 128)] = _assemble(outs, row8a)
        return carry

    def ocopy(t):
        return pltpu.make_async_copy(out_s.at[t % 2], out_h.at[pl.ds(t * TQ, TQ), :], osems.at[t % 2])

    for t in range(NC):
        lax.fori_loop(4 * t, 4 * t + 4, a_body, 0)
        oa = jnp.dot(woT_s[0], oA_s[...].astype(BF16), preferred_element_type=F32)
        ob = jnp.dot(woT_s[1], oB_s[:, pl.ds(t * TQ, TQ)].astype(BF16), preferred_element_type=F32)
        oT = jnp.concatenate([oa, ob], axis=0)
        if t >= 2:
            ocopy(t - 2).wait()
        out_s[t % 2] = oT.T.astype(BF16)
        ocopy(t).start()
    ocopy(NC - 2).wait()
    ocopy(NC - 1).wait()


def build(name="k2"):
    scratch = [
        pltpu.VMEM((D, S), BF16),
        pltpu.VMEM((D, S), BF16),
        pltpu.VMEM((D, 3 * D), BF16),
        pltpu.VMEM((D, D), BF16),
        pltpu.VMEM((2, D, D), BF16),
        pltpu.VMEM((2, DH, D), BF16),
        pltpu.VMEM((640, D), BF16),
        pltpu.VMEM((640, D), BF16),
        pltpu.VMEM((D, D), BF16),
        pltpu.VMEM((2, D, D), BF16),
        pltpu.VMEM((640, S), BF16),
        pltpu.VMEM((7, S, 128), BF16),
        pltpu.VMEM((4, 24, S), F32),
        pltpu.VMEM((2, S, TQ), F32),
        pltpu.VMEM((2, 8, TQ), F32),
        pltpu.VMEM((D, S), F32),
        pltpu.VMEM((NG, S + 256, 128), BF16),
        pltpu.VMEM((D, S + 256), F32),
        pltpu.VMEM((2, 4, 384, 128), F32),
        pltpu.VMEM((2, 4, 8, 128), F32),
        pltpu.VMEM((D, TQ), F32),
        pltpu.VMEM((2, TQ, 2 * D), BF16),
        pltpu.SemaphoreType.DMA((11,)),
        pltpu.SemaphoreType.DMA((2,)),
    ]
    any_spec = pl.BlockSpec(memory_space=pl.ANY)
    return pl.pallas_call(
        kernel_body,
        out_shape=jax.ShapeDtypeStruct((S, 2 * D), BF16),
        in_specs=[any_spec] * 8,
        out_specs=any_spec,
        scratch_shapes=scratch,
        name=name,
        compiler_params=pltpu.CompilerParams(vmem_limit_bytes=110 * 1024 * 1024),
    )


@jax.jit
def pallas_concat_heads__sliding_block__grouped_kv_mqa__prompt_kernel(
    A_x: jax.Array,
    A_wqkv: jax.Array,
    A_wo: jax.Array,
    B_x: jax.Array,
    B_wq: jax.Array,
    B_wk: jax.Array,
    B_wv: jax.Array,
    B_wo: jax.Array,
):
    out = build()(A_x[0].T, A_wqkv, A_wo, B_x[0].T, B_wq, B_wk.T, B_wv.T, B_wo)
    return out.reshape(1, S, 2 * D)
```

```python
import contextlib
import functools
import jax
import jax.numpy as jnp
import numpy as np
from jax import lax
from jax.experimental import pallas as pl
from jax.experimental.pallas import tpu as pltpu

S = 2048
D = 576
H = 32
DH = 18
NG = 5
TQ = 512
NC = S // TQ
NEG = -1e30
QSCALE = float(DH ** -0.5 * np.log2(np.e))
F32 = jnp.float32
BF16 = jnp.bfloat16
I32 = jnp.int32
_NEG_BITS = int(np.array([NEG], dtype=np.float32).view(np.uint32)[0] >> 16)
NEG2 = int(np.array([(_NEG_BITS << 16) | _NEG_BITS], dtype=np.uint32).view(np.int32)[0])


def _pad_group_rows(wt):
    n = wt.shape[1]
    parts = []
    for g in range(NG):
        lo = 126 * g
        hi = min(lo + 126, D)
        parts.append(wt[lo:hi])
        parts.append(jnp.zeros((128 - (hi - lo), n), wt.dtype))
    return jnp.concatenate(parts, axis=0)


def _assemble(o, row8):
    def sel(k, a, b):
        return jnp.where(row8 < k, a, b)
    return jnp.concatenate([
        o[0][0:8], o[0][8:16], sel(2, o[0][16:24], o[1][0:8]),
        o[1][8:16], sel(4, o[1][16:24], o[2][0:8]),
        o[2][8:16], sel(6, o[2][16:24], o[3][0:8]),
        o[3][8:16], o[3][16:24]], axis=0)


def _lrow(jj):
    return 23 if jj < 3 else 0


def make_body(scopes=False, UB=8, QPI=2, DMAALL=True, PR1=0, PR2=1, FLAT=1):
    def scope(n):
        if scopes:
            return jax.named_scope(n)
        return contextlib.nullcontext()

    def kernel_body(axT_h, awqkv_h, awo_h, bxT_h, bwq_h, bwkT_h, bwvT_h, bwo_h,
                    out_h,
                    xa_s, xb_s, wqkv_s, wq_s, wo_s, wkv_s,
                    wqT_s, wT_s, woT_s, wkvT_s, qT_s, krep_s, vTb_s, sB_s, mB_s, oB_s,
                    qTa_s, kA_s, vTa_s, sA_s, mA_s, oA_s, out_s, sems, xsems, osems):

        def cp(src, dst, i):
            return pltpu.make_async_copy(src, dst, sems.at[i])

        def xbcopy(c):
            cols = pl.ds(pl.multiple_of(c * TQ, TQ), TQ)
            return pltpu.make_async_copy(bxT_h.at[:, cols], xb_s.at[:, cols], xsems.at[c])

        c_wq = cp(bwq_h, wq_s, 0)
        c_wk = cp(bwkT_h, wkv_s.at[0], 1)
        c_wv = cp(bwvT_h, wkv_s.at[1], 2)
        c_wob = cp(bwo_h, wo_s.at[1], 3)
        c_wqkv = cp(awqkv_h, wqkv_s, 4)
        c_xa = cp(axT_h, xa_s, 5)
        c_woa = cp(awo_h, wo_s.at[0], 6)

        with scope('Bprep'):
            c_wk.start(priority=PR1)
            c_wv.start(priority=PR1)
            xbcopy(0).start(priority=PR1)
            c_wq.start(priority=PR1)
            if DMAALL:
                for c in range(1, NC):
                    xbcopy(c).start(priority=PR1)
                c_wqkv.start(priority=PR2)
                c_wob.start(priority=PR2)
                c_woa.start(priority=PR2)
                c_xa.start(priority=PR2)
            c_wk.wait()
            c_wv.wait()
            wkT = wkv_s[0].astype(F32)
            wvT = wkv_s[1].astype(F32)
            z6 = jnp.zeros((6, D), F32)
            wkvT_s[...] = jnp.concatenate([wkT, z6, wvT, z6], axis=0).astype(BF16)
            c_wq.wait()
            wqT_s[...] = wq_s[...].T

        def b_proj(c, carry):
            row24 = lax.broadcasted_iota(I32, (24, TQ), 0)
            cols = pl.ds(pl.multiple_of(c * TQ, TQ), TQ)
            xbcopy(c).wait()

            if not DMAALL:
                @pl.when(c + 1 < NC)
                def _():
                    xbcopy(c + 1).start()

                @pl.when(c == 1)
                def _():
                    c_wqkv.start()
                    c_wob.start()
                    c_woa.start()
            xT = xb_s[:, cols]
            kvT = jnp.dot(wkvT_s[...], xT, preferred_element_type=F32)
            k = kvT[0:DH]
            kr = jnp.concatenate([k] * 7 + [jnp.zeros((2, TQ), F32)], axis=0).astype(BF16).T
            krep_s[pl.ds(pl.multiple_of(c * (TQ // 2), TQ // 2), TQ // 2), :] = pltpu.bitcast(kr, I32)
            vT = kvT[24:48].astype(BF16).astype(F32)
            for jj in range(4):
                off = 2 * jj
                if off:
                    vv = jnp.concatenate([jnp.zeros((off, TQ), F32), vT[0:24 - off]], axis=0)
                else:
                    vv = vT
                vTb_s[jj, :, cols] = jnp.where(row24 == _lrow(jj), 1.0, vv)
            qT = jnp.dot(wqT_s[...], xT, preferred_element_type=F32) * QSCALE
            qT_s[:, cols] = _pad_group_rows(qT).astype(BF16)
            return carry

        with scope('Bproj'):
            lax.fori_loop(0, NC, b_proj, 0)
        if not DMAALL:
            c_xa.start()

        NCH = S // 128

        def b_qk_pre(it):
            h = it % H
            j = h % 7
            lane = lax.broadcasted_iota(I32, (8, 128), 1)
            return jnp.where((lane >= DH * j) & (lane < DH * j + DH), I32(-1), I32(0))

        def b_qk_chunk(it, c, slot, m, kmask):
            qt = it // H
            g = (it % H) // 7
            w = qT_s[pl.ds(pl.multiple_of(g * 128, 128), 128), pl.ds(pl.multiple_of(qt * TQ, TQ), TQ)]
            ki = krep_s[pl.ds(c * 64, 64), :].reshape(8, 8, 128) & kmask
            k = pltpu.bitcast(ki.reshape(64, 128), BF16)
            s = jnp.dot(k, w, preferred_element_type=F32)
            sB_s[slot, pl.ds(c * 128, 128), :] = s
            mm = jnp.max(s.reshape(16, 8, TQ), axis=0)
            return mm if m is None else jnp.maximum(m, mm)

        def b_fin_m(m8, slot):
            mB_s[slot] = jnp.broadcast_to(jnp.max(m8, axis=0, keepdims=True), (8, TQ))

        def b_pv_chunk(c, slot, jj, m, acc):
            p = jnp.exp2(sB_s[slot, pl.ds(c * 128, 128), :] - m).astype(BF16)
            o = jnp.dot(vTb_s[jj, :, pl.ds(c * 128, 128)], p, preferred_element_type=F32)
            return o if acc is None else acc + o

        NIT = NC * H

        def b_body(i, carry):
            row8 = lax.broadcasted_iota(I32, (8, TQ), 0)
            for uu in range(UB // 4):
                outs = []
                for jj in range(4):
                    it = i * UB + uu * 4 + jj
                    slot = jj % 2
                    itn = jnp.minimum(it + 1, NIT - 1)
                    mcur = mB_s[slot][0:1, :]
                    kmask = b_qk_pre(itn)
                    mn = None
                    acc = None
                    for c in range(NCH):
                        mn = b_qk_chunk(itn, c, 1 - slot, mn, kmask)
                        acc = b_pv_chunk(c, slot, jj, mcur, acc)
                    b_fin_m(mn, 1 - slot)
                    lr = _lrow(jj)
                    outs.append(acc * (1.0 / acc[lr:lr + 1, :]))
                iu = i * (UB // 4) + uu
                qt = iu // 8
                u = iu % 8
                oB_s[pl.ds(pl.multiple_of(u * 72, 8), 72),
                     pl.ds(pl.multiple_of(qt * TQ, TQ), TQ)] = _assemble(outs, row8)
            return carry

        with scope('Bpre'):
            c_wob.wait()
            c_wqkv.wait()
            c_woa.wait()
            wT_s[...] = wqkv_s[...].T
            woT_s[0] = wo_s[0].T
            woT_s[1] = wo_s[1].T
            lane = lax.broadcasted_iota(I32, (1, 128), 1)
            for g in range(NG):
                kA_s[g, 0:256, :] = jnp.broadcast_to(
                    jnp.where(lane >= 126, 1.0, 0.0), (256, 128)).astype(BF16)
            vTa_s[:, 0:256] = jnp.zeros((D, 256), F32)
            m = None
            kmask0 = b_qk_pre(0)
            for c in range(NCH):
                m = b_qk_chunk(0, c, 0, m, kmask0)
            b_fin_m(m, 0)
        with scope('Battn'):
            lax.fori_loop(0, NIT // UB, b_body, 0)

        def a_proj(c, carry):
            cols = pl.ds(pl.multiple_of(c * TQ, TQ), TQ)
            pcols = pl.ds(pl.multiple_of(256 + c * TQ, 256), TQ)
            xT = xa_s[:, cols]
            kT = jnp.dot(wT_s[D:2 * D, :], xT, preferred_element_type=F32)
            kT = _pad_group_rows(kT).astype(BF16)
            for g in range(NG):
                kA_s[g, pcols, :] = kT[128 * g:128 * (g + 1)].T
            qT = jnp.dot(wT_s[0:D, :], xT, preferred_element_type=F32) * QSCALE
            qTa_s[:, cols] = pltpu.bitcast(_pad_group_rows(qT).astype(BF16), I32)
            vT = jnp.dot(wT_s[2 * D:3 * D, :], xT, preferred_element_type=F32)
            vTa_s[:, pcols] = vT.astype(BF16).astype(F32)
            return carry

        with scope('Aproj'):
            c_xa.wait()
            lax.fori_loop(0, NC, a_proj, 0)

        def a_qk_head(qt, h, slot, hh):
            r128 = lax.broadcasted_iota(I32, (128, 128), 0)
            l128 = lax.broadcasted_iota(I32, (128, 128), 1)
            r8 = lax.broadcasted_iota(I32, (8, 128), 0)
            g, j = h // 7, h % 7
            q0 = pl.multiple_of(qt * 128, 128)
            lo, hi = 9 * j, 9 * j + 9
            blocks = []
            for b in range(8):
                r0 = 8 * b
                if r0 + 8 <= lo or r0 >= hi:
                    blk = jnp.zeros((8, 128), I32)
                else:
                    blk = qTa_s[pl.ds(64 * g + r0, 8), pl.ds(q0, 128)]
                    if not (r0 >= lo and r0 + 8 <= hi):
                        blk = jnp.where((r8 + r0 >= lo) & (r8 + r0 < hi), blk, I32(0))
                if b == 7:
                    blk = jnp.where(r8 == 7, I32(NEG2), blk)
                blocks.append(blk)
            w = pltpu.bitcast(jnp.concatenate(blocks, axis=0), BF16)
            s = jnp.dot(kA_s[g, pl.ds(q0, 384), :], w, preferred_element_type=F32)
            s0 = jnp.where(r128 > l128, s[0:128], NEG)
            s1 = s[128:256]
            s2 = jnp.where(r128 <= l128, s[256:384], NEG)
            sA_s[slot, hh, 0:128, :] = s0
            sA_s[slot, hh, 128:256, :] = s1
            sA_s[slot, hh, 256:384, :] = s2
            mm = jnp.maximum(jnp.maximum(s0, s1), s2)
            mm = jnp.max(mm.reshape(16, 8, 128), axis=0)
            mm = jnp.max(mm, axis=0, keepdims=True)
            mA_s[slot, hh] = jnp.broadcast_to(mm, (8, 128))

        def a_pv_tile(qt, h, slot, hh, t, acc):
            r24 = lax.broadcasted_iota(I32, (24, 128), 0)
            q0 = pl.multiple_of(qt * 128 + 128 * t, 128)
            r0 = (DH * h) // 8 * 8
            lr = _lrow(h % 4)
            m = mA_s[slot, hh][0:1, :]
            p = jnp.exp2(sA_s[slot, hh, 128 * t:128 * (t + 1), :] - m).astype(BF16)
            v = jnp.where(r24 == lr, 1.0, vTa_s[r0:r0 + 24, pl.ds(q0, 128)])
            o = jnp.dot(v, p, preferred_element_type=F32)
            return o if acc is None else acc + o

        NQT = S // 128

        def a_qtile(qt, nper=4):
            row8a = lax.broadcasted_iota(I32, (8, 128), 0)
            for s in range(8):
                slot = s % 2
                if s < 7:
                    nqt, nh0 = qt, (s + 1) * 4
                else:
                    nqt, nh0 = jnp.minimum(qt + 1, NQT - 1), 0
                for hh in range(4):
                    a_qk_head(nqt, nh0 + hh, 1 - slot, hh)
                accs = [None] * 4
                for t in range(3):
                    for hh in range(4):
                        accs[hh] = a_pv_tile(qt, s * 4 + hh, slot, hh, t, accs[hh])
                outs = [accs[hh] * (1.0 / accs[hh][_lrow(hh):_lrow(hh) + 1, :]) for hh in range(4)]
                oA_s[pl.ds(72 * s, 72), pl.ds(pl.multiple_of((qt % nper) * 128, 128), 128)] = _assemble(outs, row8a)

        def ocopy(t, part):
            rows = pl.ds(pl.multiple_of(t * TQ, TQ), TQ)
            cols = pl.ds(0, 640) if part == 0 else pl.ds(640, 512)
            return pltpu.make_async_copy(out_s.at[t % 2, :, cols], out_h.at[rows, cols], osems.at[t % 2, part])

        def a_tile(t, carry):
            cols = pl.ds(pl.multiple_of(t * TQ, TQ), TQ)
            ob = oB_s[:, cols].astype(BF16)

            @pl.when(t >= 2)
            def _():
                ocopy(t - 2, 1).wait()
                ocopy(t - 2, 0).wait()
            for i in range(5, 9):
                r0 = 64 + 128 * (i - 5)
                r = jnp.dot(woT_s[1, r0:r0 + 128, :], ob, preferred_element_type=F32)
                out_s[t % 2, :, 128 * i:128 * (i + 1)] = r.astype(BF16).T
            ocopy(t, 1).start()
            rb = jnp.dot(woT_s[1, 0:64, :], ob, preferred_element_type=F32).astype(BF16)
            if QPI == 4:
                for qq in range(4):
                    a_qtile(4 * t + qq)
            else:
                def body(i, c):
                    for qq in range(QPI):
                        a_qtile(4 * t + i * QPI + qq)
                    return c
                lax.fori_loop(0, 4 // QPI, body, 0)
            oa = oA_s[...].astype(BF16)
            ra = jnp.dot(woT_s[0, 512:576, :], oa, preferred_element_type=F32).astype(BF16)
            out_s[t % 2, :, 512:640] = jnp.concatenate([ra, rb], axis=0).T
            for i in range(4):
                r = jnp.dot(woT_s[0, 128 * i:128 * (i + 1), :], oa, preferred_element_type=F32)
                out_s[t % 2, :, 128 * i:128 * (i + 1)] = r.astype(BF16).T
            ocopy(t, 0).start()
            return carry

        TF = 256

        def fcopy(t):
            rows = pl.ds(pl.multiple_of(t * TF, TF), TF)
            return pltpu.make_async_copy(out_s.at[t % 2, 0:TF], out_h.at[rows, :], osems.at[t % 2, 0])

        def f_tile(t, carry):
            cols = pl.ds(pl.multiple_of(t * TF, TF), TF)
            ob = oB_s[:, cols].astype(BF16)

            @pl.when(t >= 2)
            def _():
                fcopy(t - 2).wait()
            for i in range(5, 9):
                r0 = 64 + 128 * (i - 5)
                r = jnp.dot(woT_s[1, r0:r0 + 128, :], ob, preferred_element_type=F32)
                out_s[t % 2, 0:TF, 128 * i:128 * (i + 1)] = r.astype(BF16).T
            rb = jnp.dot(woT_s[1, 0:64, :], ob, preferred_element_type=F32).astype(BF16)
            for qq in range(2):
                a_qtile(2 * t + qq, 2)
            oa = oA_s[:, 0:TF].astype(BF16)
            ra = jnp.dot(woT_s[0, 512:576, :], oa, preferred_element_type=F32).astype(BF16)
            out_s[t % 2, 0:TF, 512:640] = jnp.concatenate([ra, rb], axis=0).T
            for i in range(4):
                r = jnp.dot(woT_s[0, 128 * i:128 * (i + 1), :], oa, preferred_element_type=F32)
                out_s[t % 2, 0:TF, 128 * i:128 * (i + 1)] = r.astype(BF16).T
            fcopy(t).start()
            return carry

        with scope('Aattn'):
            for hh in range(4):
                a_qk_head(0, hh, 0, hh)
            if FLAT:
                lax.fori_loop(0, S // TF, f_tile, 0)
            else:
                lax.fori_loop(0, NC, a_tile, 0)
        if FLAT:
            fcopy(S // TF - 2).wait()
            fcopy(S // TF - 1).wait()
        else:
            for t in (NC - 2, NC - 1):
                ocopy(t, 1).wait()
                ocopy(t, 0).wait()

    return kernel_body


def build(name="k5", FLAGS=None, **kw):
    scratch = [
        pltpu.VMEM((D, S), BF16),
        pltpu.VMEM((D, S), BF16),
        pltpu.VMEM((D, 3 * D), BF16),
        pltpu.VMEM((D, D), BF16),
        pltpu.VMEM((2, D, D), BF16),
        pltpu.VMEM((2, DH, D), BF16),
        pltpu.VMEM((D, D), BF16),
        pltpu.VMEM((3 * D, D), BF16),
        pltpu.VMEM((2, D, D), BF16),
        pltpu.VMEM((48, D), BF16),
        pltpu.VMEM((640, S), BF16),
        pltpu.VMEM((S // 2, 128), I32),
        pltpu.VMEM((4, 24, S), F32),
        pltpu.VMEM((2, S, TQ), F32),
        pltpu.VMEM((2, 8, TQ), F32),
        pltpu.VMEM((D, S), F32),
        pltpu.VMEM((320, S), I32),
        pltpu.VMEM((NG, S + 256, 128), BF16),
        pltpu.VMEM((D, S + 256), F32),
        pltpu.VMEM((2, 4, 384, 128), F32),
        pltpu.VMEM((2, 4, 8, 128), F32),
        pltpu.VMEM((D, TQ), F32),
        pltpu.VMEM((2, TQ, 2 * D), BF16),
        pltpu.SemaphoreType.DMA((7,)),
        pltpu.SemaphoreType.DMA((NC,)),
        pltpu.SemaphoreType.DMA((2, 2)),
    ]
    any_spec = pl.BlockSpec(memory_space=pl.ANY)
    return pl.pallas_call(
        make_body(**kw),
        out_shape=jax.ShapeDtypeStruct((S, 2 * D), BF16),
        in_specs=[any_spec] * 8,
        out_specs=any_spec,
        scratch_shapes=scratch,
        name=name,
        compiler_params=pltpu.CompilerParams(vmem_limit_bytes=110 * 1024 * 1024,
                                             flags=({'XLA_TPU_EVENLY_DISTRIBUTE_CRITICAL_NODES': True} if FLAGS else None)),
    )


@jax.jit
def pallas_concat_heads__sliding_block__grouped_kv_mqa__prompt_kernel(
    A_x: jax.Array,
    A_wqkv: jax.Array,
    A_wo: jax.Array,
    B_x: jax.Array,
    B_wq: jax.Array,
    B_wk: jax.Array,
    B_wv: jax.Array,
    B_wo: jax.Array,
):
    out = build()(A_x[0].T, A_wqkv, A_wo, B_x[0].T, B_wq, B_wk.T, B_wv.T, B_wo)
    return out.reshape(1, S, 2 * D)
```

```python
import contextlib
import functools
import jax
import jax.numpy as jnp
import numpy as np
from jax import lax
from jax.experimental import pallas as pl
from jax.experimental.pallas import tpu as pltpu

S = 2048
D = 576
H = 32
DH = 18
NG = 5
TQ = 512
NC = S // TQ
NEG = -1e30
QSCALE = float(DH ** -0.5 * np.log2(np.e))
F32 = jnp.float32
BF16 = jnp.bfloat16
I32 = jnp.int32
_NEG_BITS = int(np.array([NEG], dtype=np.float32).view(np.uint32)[0] >> 16)
NEG2 = int(np.array([(_NEG_BITS << 16) | _NEG_BITS], dtype=np.uint32).view(np.int32)[0])


def _pad_group_rows(wt):
    n = wt.shape[1]
    parts = []
    for g in range(NG):
        lo = 126 * g
        hi = min(lo + 126, D)
        parts.append(wt[lo:hi])
        parts.append(jnp.zeros((128 - (hi - lo), n), wt.dtype))
    return jnp.concatenate(parts, axis=0)


def _assemble(o, row8):
    def sel(k, a, b):
        return jnp.where(row8 < k, a, b)
    return jnp.concatenate([
        o[0][0:8], o[0][8:16], sel(2, o[0][16:24], o[1][0:8]),
        o[1][8:16], sel(4, o[1][16:24], o[2][0:8]),
        o[2][8:16], sel(6, o[2][16:24], o[3][0:8]),
        o[3][8:16], o[3][16:24]], axis=0)


def _lrow(jj):
    return 23 if jj < 3 else 0


def make_body(scopes=False, UB=8, QPI=2, DMAALL=True, PR1=0, PR2=1, FLAT=1, LAG=1, KTAB=0, CUT=192, MERGE=0, KVAR=0, OPOS=0):
    def scope(n):
        if scopes:
            return jax.named_scope(n)
        return contextlib.nullcontext()

    def kernel_body(axT_h, awqkv_h, awo_h, bxT_h, bwq_h, bwkT_h, bwvT_h, bwo_h,
                    out_h,
                    xa_s, xb_s, wqkv_s, wq_s, wo_s, wkv_s,
                    wqT_s, wT_s, woT_s, wkvT_s, qT_s, krep_s, vTb_s, pad_s, sB_s, mB_s, oB_s,
                    qTa_s, kA_s, vTa_s, sA_s, mA_s, oA_s, out_s, kmask_s, kvar_s, sems, xsems, osems):

        def cp(src, dst, i):
            return pltpu.make_async_copy(src, dst, sems.at[i])

        def xbcopy(c):
            cols = pl.ds(pl.multiple_of(c * TQ, TQ), TQ)
            return pltpu.make_async_copy(bxT_h.at[:, cols], xb_s.at[:, cols], xsems.at[c])

        c_wq = cp(bwq_h, wq_s, 0)
        c_wk = cp(bwkT_h, wkv_s.at[0], 1)
        c_wv = cp(bwvT_h, wkv_s.at[1], 2)
        c_wob = cp(bwo_h, wo_s.at[1], 3)
        c_wqkv = cp(awqkv_h, wqkv_s, 4)
        c_xa = cp(axT_h, xa_s, 5)
        c_woa = cp(awo_h, wo_s.at[0], 6)

        with scope('Bprep'):
            c_wk.start(priority=PR1)
            c_wv.start(priority=PR1)
            c_wq.start(priority=PR1)
            xbcopy(0).start(priority=PR1)
            if DMAALL:
                for c in range(1, NC):
                    xbcopy(c).start(priority=PR1)
                c_wqkv.start(priority=PR2)
                c_wob.start(priority=PR2)
                c_woa.start(priority=PR2)
                c_xa.start(priority=PR2)
            lane8 = lax.broadcasted_iota(I32, (8, 128), 1)
            for j in range(7):
                kmask_s[j] = jnp.where((lane8 >= DH * j) & (lane8 < DH * j + DH), I32(-1), I32(0))
            c_wk.wait()
            c_wv.wait()
            wkT = wkv_s[0].astype(F32)
            wvT = wkv_s[1].astype(F32)
            z6 = jnp.zeros((6, D), F32)
            wkvT_s[...] = jnp.concatenate([wkT, z6, wvT, z6], axis=0).astype(BF16)
            c_wq.wait()
            wqT_s[...] = wq_s[...].T

        def b_proj(c, carry):
            row24 = lax.broadcasted_iota(I32, (24, TQ), 0)
            cols = pl.ds(pl.multiple_of(c * TQ, TQ), TQ)
            xbcopy(c).wait()

            if not DMAALL:
                @pl.when(c + 1 < NC)
                def _():
                    xbcopy(c + 1).start()

                @pl.when(c == 1)
                def _():
                    c_wqkv.start()
                    c_wob.start()
                    c_woa.start()
            xT = xb_s[:, cols]
            kvT = jnp.dot(wkvT_s[...], xT, preferred_element_type=F32)
            k = kvT[0:DH]
            kr = jnp.concatenate([k] * 7 + [jnp.zeros((2, TQ), F32)], axis=0).astype(BF16).T
            krows = pl.ds(pl.multiple_of(c * (TQ // 2), TQ // 2), TQ // 2)
            krep_s[krows, :] = pltpu.bitcast(kr, I32)
            if KVAR:
                ki = krep_s[krows, :]
                lane1 = lax.broadcasted_iota(I32, (1, 128), 1)
                for j in range(7):
                    kvar_s[j, krows, :] = ki & jnp.where(
                        (lane1 >= DH * j) & (lane1 < DH * j + DH), I32(-1), I32(0))
            vT = kvT[24:48].astype(BF16).astype(F32)
            for jj in range(4):
                off = 2 * jj
                if off:
                    vv = jnp.concatenate([jnp.zeros((off, TQ), F32), vT[0:24 - off]], axis=0)
                else:
                    vv = vT
                vTb_s[jj, :, cols] = jnp.where(row24 == _lrow(jj), 1.0, vv)
            qT = jnp.dot(wqT_s[...], xT, preferred_element_type=F32) * QSCALE
            qT_s[:, cols] = _pad_group_rows(qT).astype(BF16)
            return carry

        with scope('Bproj'):
            lax.fori_loop(0, NC, b_proj, 0)
        if not DMAALL:
            c_xa.start()

        NCH = S // 128

        def b_qk_pre(it):
            h = it % H
            j = h % 7
            if KTAB:
                return kmask_s[j]
            lane = lax.broadcasted_iota(I32, (8, 128), 1)
            return jnp.where((lane >= DH * j) & (lane < DH * j + DH), I32(-1), I32(0))

        def b_qk_chunk(it, c, slot, m, kmask):
            qt = it // H
            g = (it % H) // 7
            w = qT_s[pl.ds(pl.multiple_of(g * 128, 128), 128), pl.ds(pl.multiple_of(qt * TQ, TQ), TQ)]
            if KVAR:
                k = pltpu.bitcast(kvar_s[(it % H) % 7, pl.ds(c * 64, 64), :], BF16)
            else:
                ki = krep_s[pl.ds(c * 64, 64), :].reshape(8, 8, 128) & kmask
                k = pltpu.bitcast(ki.reshape(64, 128), BF16)
            s = jnp.dot(k, w, preferred_element_type=F32)
            sB_s[slot, pl.ds(c * 128, 128), :] = s
            mm = jnp.max(s.reshape(16, 8, TQ), axis=0)
            return mm if m is None else jnp.maximum(m, mm)

        def b_fin_m(m8, slot):
            mB_s[slot] = jnp.broadcast_to(jnp.max(m8, axis=0, keepdims=True), (8, TQ))

        def b_pv_chunk(c, slot, jj, m, acc):
            p = jnp.exp2(sB_s[slot, pl.ds(c * 128, 128), :] - m).astype(BF16)
            o = jnp.dot(vTb_s[jj, :, pl.ds(c * 128, 128)], p, preferred_element_type=F32)
            return o if acc is None else acc + o

        NIT = NC * H

        def b_body(i, carry):
            row8 = lax.broadcasted_iota(I32, (8, TQ), 0)
            seq = [(st, c) for st in range(UB) for c in range(NCH)]
            mns, ms, accs, kmasks, outs = {}, {}, {}, {}, {}
            for n in range(len(seq) + LAG):
                if n < len(seq):
                    st, c = seq[n]
                    itn = jnp.minimum(i * UB + st + 1, NIT - 1)
                    if c == 0:
                        kmasks[st] = b_qk_pre(itn)
                    mns[st] = b_qk_chunk(itn, c, 1 - st % 2, mns.get(st), kmasks[st])
                if n >= LAG:
                    st, c = seq[n - LAG]
                    jj = st % 4
                    if c == 0:
                        ms[st] = (mB_s[0][0:1, :] if st == 0
                                  else jnp.max(mns[st - 1], axis=0, keepdims=True))
                    accs[st] = b_pv_chunk(c, st % 2, jj, ms[st], accs.get(st))
                    if c == NCH - 1:
                        lr = _lrow(jj)
                        outs[jj] = accs[st] * (1.0 / accs[st][lr:lr + 1, :])
                        if jj == 3:
                            iu = i * (UB // 4) + st // 4
                            qt = iu // 8
                            u = iu % 8
                            oB_s[pl.ds(pl.multiple_of(u * 72, 8), 72),
                                 pl.ds(pl.multiple_of(qt * TQ, TQ), TQ)] = _assemble(outs, row8)
            b_fin_m(mns[UB - 1], 0)
            return carry

        def a_proj(c, carry):
            cols = pl.ds(pl.multiple_of(c * TQ, TQ), TQ)
            pcols = pl.ds(pl.multiple_of(256 + c * TQ, 256), TQ)
            xT = xa_s[:, cols]
            kT = jnp.dot(wT_s[D:2 * D, :], xT, preferred_element_type=F32)
            kT = _pad_group_rows(kT).astype(BF16)
            for g in range(NG):
                kA_s[g, pcols, :] = kT[128 * g:128 * (g + 1)].T
            qT = jnp.dot(wT_s[0:D, :], xT, preferred_element_type=F32) * QSCALE
            qTa_s[:, cols] = pltpu.bitcast(_pad_group_rows(qT).astype(BF16), I32)
            vT = jnp.dot(wT_s[2 * D:3 * D, :], xT, preferred_element_type=F32)
            vTa_s[:, pcols] = vT.astype(BF16).astype(F32)
            return carry

        with scope('Bpre'):
            c_wob.wait()
            c_wqkv.wait()
            c_woa.wait()
            wT_s[...] = wqkv_s[...].T
            woT_s[0] = wo_s[0].T
            woT_s[1] = wo_s[1].T
            lane = lax.broadcasted_iota(I32, (1, 128), 1)
            for g in range(NG):
                kA_s[g, 0:256, :] = jnp.broadcast_to(
                    jnp.where(lane >= 126, 1.0, 0.0), (256, 128)).astype(BF16)
            vTa_s[:, 0:256] = jnp.zeros((D, 256), F32)
            m = None
            kmask0 = b_qk_pre(0)
            for c in range(NCH):
                m = b_qk_chunk(0, c, 0, m, kmask0)
            b_fin_m(m, 0)
            if MERGE:
                c_xa.wait()
                a_proj(0, 0)
        with scope('Battn'):
            lax.fori_loop(0, NIT // UB, b_body, 0)

        with scope('Aproj'):
            if MERGE:
                lax.fori_loop(1, NC, a_proj, 0)
            else:
                c_xa.wait()
                lax.fori_loop(0, NC, a_proj, 0)

        def a_wts(qt, h):
            r8 = lax.broadcasted_iota(I32, (8, 128), 0)
            g, j = h // 7, h % 7
            q0 = pl.multiple_of(qt * 128, 128)
            lo, hi = 9 * j, 9 * j + 9
            blocks = []
            for b in range(8):
                r0 = 8 * b
                if r0 + 8 <= lo or r0 >= hi:
                    blk = jnp.zeros((8, 128), I32)
                else:
                    blk = qTa_s[pl.ds(64 * g + r0, 8), pl.ds(q0, 128)]
                    if not (r0 >= lo and r0 + 8 <= hi):
                        blk = jnp.where((r8 + r0 >= lo) & (r8 + r0 < hi), blk, I32(0))
                if b == 7:
                    blk = jnp.where(r8 == 7, I32(NEG2), blk)
                blocks.append(blk)
            return pltpu.bitcast(jnp.concatenate(blocks, axis=0), BF16)

        def a_qk_rows(qt, h, slot, hh, r0, r1, w, mm):
            g = h // 7
            q0 = pl.multiple_of(qt * 128, 128)
            s = jnp.dot(kA_s[g, pl.ds(q0 + r0, r1 - r0), :], w, preferred_element_type=F32)
            r64 = lax.broadcasted_iota(I32, (64, 128), 0)
            l64 = lax.broadcasted_iota(I32, (64, 128), 1)
            for a in range(r0, r1, 64):
                blk = s[a - r0:a - r0 + 64]
                if a < 128:
                    blk = jnp.where(r64 + a > l64, blk, NEG)
                elif a >= 256:
                    blk = jnp.where(r64 + (a - 256) <= l64, blk, NEG)
                sA_s[slot, hh, a:a + 64, :] = blk
                mm = blk if mm is None else jnp.maximum(mm, blk)
            return mm

        def a_fin_m(mm, slot, hh):
            mm = jnp.max(mm.reshape(8, 8, 128), axis=0)
            mA_s[slot, hh] = jnp.broadcast_to(jnp.max(mm, axis=0, keepdims=True), (8, 128))

        def a_qk_head(qt, h, slot, hh):
            a_fin_m(a_qk_rows(qt, h, slot, hh, 0, 384, a_wts(qt, h), None), slot, hh)

        def a_pv_tile(qt, h, slot, hh, t, acc):
            r24 = lax.broadcasted_iota(I32, (24, 128), 0)
            q0 = pl.multiple_of(qt * 128 + 128 * t, 128)
            r0 = (DH * h) // 8 * 8
            lr = _lrow(h % 4)
            m = mA_s[slot, hh][0:1, :]
            p = jnp.exp2(sA_s[slot, hh, 128 * t:128 * (t + 1), :] - m).astype(BF16)
            v = jnp.where(r24 == lr, 1.0, vTa_s[r0:r0 + 24, pl.ds(q0, 128)])
            o = jnp.dot(v, p, preferred_element_type=F32)
            return o if acc is None else acc + o

        NQT = S // 128

        def a_qtile(qt, oslot, qq, hook=None):
            row8a = lax.broadcasted_iota(I32, (8, 128), 0)
            for s in range(8):
                slot = s % 2
                if s < 7:
                    nqt, nh0 = qt, (s + 1) * 4
                else:
                    nqt, nh0 = jnp.minimum(qt + 1, NQT - 1), 0
                ws = [a_wts(nqt, nh0 + hh) for hh in range(4)]
                mms = [a_qk_rows(nqt, nh0 + hh, 1 - slot, hh, 0, CUT, ws[hh], None) for hh in range(4)]
                accs = [a_pv_tile(qt, s * 4 + hh, slot, hh, 0, None) for hh in range(4)]
                mms = [a_qk_rows(nqt, nh0 + hh, 1 - slot, hh, CUT, 384, ws[hh], mms[hh]) for hh in range(4)]
                for t in (1, 2):
                    accs = [a_pv_tile(qt, s * 4 + hh, slot, hh, t, accs[hh]) for hh in range(4)]
                for hh in range(4):
                    a_fin_m(mms[hh], 1 - slot, hh)
                outs = [accs[hh] * (1.0 / accs[hh][_lrow(hh):_lrow(hh) + 1, :]) for hh in range(4)]
                oA_s[oslot, pl.ds(72 * s, 72), pl.ds(qq * 128, 128)] = _assemble(outs, row8a)
                if hook is not None:
                    hook(s)

        TF = 256
        NT_ = S // TF

        def fcopy(t, part):
            rows = pl.ds(pl.multiple_of(t * TF, TF), TF)
            cols = pl.ds(0, 640) if part == 0 else pl.ds(640, 512)
            return pltpu.make_async_copy(out_s.at[rows, cols], out_h.at[rows, cols], osems.at[t, part])

        def out_proj(t):
            rows = pl.ds(pl.multiple_of(t * TF, TF), TF)
            ob = oB_s[:, rows].astype(BF16)
            oa = oA_s[t % 2].astype(BF16)
            for i in range(9):
                if i < 4:
                    r = jnp.dot(woT_s[0, 128 * i:128 * (i + 1), :], oa, preferred_element_type=F32)
                elif i == 4:
                    ra = jnp.dot(woT_s[0, 512:576, :], oa, preferred_element_type=F32)
                    rb = jnp.dot(woT_s[1, 0:64, :], ob, preferred_element_type=F32)
                    r = jnp.concatenate([ra, rb], axis=0)
                else:
                    r0 = 64 + 128 * (i - 5)
                    r = jnp.dot(woT_s[1, r0:r0 + 128, :], ob, preferred_element_type=F32)
                out_s[rows, 128 * i:128 * (i + 1)] = r.astype(BF16).T
                if i == 4:
                    fcopy(t, 0).start()
            fcopy(t, 1).start()

        def attn_tile(t):
            for qq in range(2):
                a_qtile(2 * t + qq, t % 2, qq)

        def f_tile(t, carry):
            if OPOS == 0:
                out_proj(t - 1)
                attn_tile(t)
            elif OPOS == 1:
                a_qtile(2 * t, t % 2, 0)
                out_proj(t - 1)
                a_qtile(2 * t + 1, t % 2, 1)
            elif OPOS == 2:
                attn_tile(t)
                out_proj(t - 1)
            else:
                a_qtile(2 * t, t % 2, 0, lambda s_: out_proj(t - 1) if s_ == OPOS - 3 else None)
                a_qtile(2 * t + 1, t % 2, 1)
            return carry

        with scope('Aattn'):
            for hh in range(4):
                a_qk_head(0, hh, 0, hh)
            attn_tile(0)
            lax.fori_loop(1, NT_, f_tile, 0)
            out_proj(NT_ - 1)
        for t in range(NT_):
            fcopy(t, 0).wait()
            fcopy(t, 1).wait()

    return kernel_body


def build(name="k7", FLAGS=None, PAD1=0, PAD2=0, **kw):
    scratch = [
        pltpu.VMEM((D, S), BF16),
        pltpu.VMEM((D, S), BF16),
        pltpu.VMEM((D, 3 * D), BF16),
        pltpu.VMEM((D, D), BF16),
        pltpu.VMEM((2, D, D), BF16),
        pltpu.VMEM((2, DH, D), BF16),
        pltpu.VMEM((D, D), BF16),
        pltpu.VMEM((3 * D, D), BF16),
        pltpu.VMEM((2, D, D), BF16),
        pltpu.VMEM((48, D), BF16),
        pltpu.VMEM((640, S), BF16),
        pltpu.VMEM((S // 2, 128), I32),
        pltpu.VMEM((4, 24, S), F32),
        pltpu.VMEM((8 + 8 * PAD1, 128), F32),
        pltpu.VMEM((2, S + 8 * PAD2, TQ), F32),
        pltpu.VMEM((2, 8, TQ), F32),
        pltpu.VMEM((D, S), F32),
        pltpu.VMEM((320, S), I32),
        pltpu.VMEM((NG, S + 256, 128), BF16),
        pltpu.VMEM((D, S + 256), F32),
        pltpu.VMEM((2, 4, 384, 128), F32),
        pltpu.VMEM((2, 4, 8, 128), F32),
        pltpu.VMEM((2, D, 256), F32),
        pltpu.VMEM((S, 2 * D), BF16),
        pltpu.VMEM((7, 8, 128), I32),
        pltpu.VMEM((7, S // 2, 128), I32),
        pltpu.SemaphoreType.DMA((7,)),
        pltpu.SemaphoreType.DMA((NC,)),
        pltpu.SemaphoreType.DMA((8, 2)),
    ]
    any_spec = pl.BlockSpec(memory_space=pl.ANY)
    return pl.pallas_call(
        make_body(**kw),
        out_shape=jax.ShapeDtypeStruct((S, 2 * D), BF16),
        in_specs=[any_spec] * 8,
        out_specs=any_spec,
        scratch_shapes=scratch,
        name=name,
        compiler_params=pltpu.CompilerParams(vmem_limit_bytes=110 * 1024 * 1024,
                                             flags=({'XLA_TPU_EVENLY_DISTRIBUTE_CRITICAL_NODES': True} if FLAGS else None)),
    )


@jax.jit
def pallas_concat_heads__sliding_block__grouped_kv_mqa__prompt_kernel(
    A_x: jax.Array,
    A_wqkv: jax.Array,
    A_wo: jax.Array,
    B_x: jax.Array,
    B_wq: jax.Array,
    B_wk: jax.Array,
    B_wv: jax.Array,
    B_wo: jax.Array,
):
    out = build()(A_x[0].T, A_wqkv, A_wo, B_x[0].T, B_wq, B_wk.T, B_wv.T, B_wo)
    return out.reshape(1, S, 2 * D)
```

```python
import contextlib
import functools
import jax
import jax.numpy as jnp
import numpy as np
from jax import lax
from jax.experimental import pallas as pl
from jax.experimental.pallas import tpu as pltpu

S = 2048
D = 576
H = 32
DH = 18
NG = 5
TQ = 512
NC = S // TQ
NEG = -1e30
QSCALE = float(DH ** -0.5 * np.log2(np.e))
F32 = jnp.float32
BF16 = jnp.bfloat16
I32 = jnp.int32
_NEG_BITS = int(np.array([NEG], dtype=np.float32).view(np.uint32)[0] >> 16)
NEG2 = int(np.array([(_NEG_BITS << 16) | _NEG_BITS], dtype=np.uint32).view(np.int32)[0])


def _pad_group_rows(wt):
    n = wt.shape[1]
    parts = []
    for g in range(NG):
        lo = 126 * g
        hi = min(lo + 126, D)
        parts.append(wt[lo:hi])
        parts.append(jnp.zeros((128 - (hi - lo), n), wt.dtype))
    return jnp.concatenate(parts, axis=0)


def _assemble(o, row8):
    def sel(k, a, b):
        return jnp.where(row8 < k, a, b)
    return jnp.concatenate([
        o[0][0:8], o[0][8:16], sel(2, o[0][16:24], o[1][0:8]),
        o[1][8:16], sel(4, o[1][16:24], o[2][0:8]),
        o[2][8:16], sel(6, o[2][16:24], o[3][0:8]),
        o[3][8:16], o[3][16:24]], axis=0)


def _lrow(jj):
    return 23 if jj < 3 else 0


def make_body(scopes=False, UB=8, QPI=2, DMAALL=True, PR1=0, PR2=1, FLAT=1, LAG=1, KTAB=0, CUT=256, MERGE=1, KVAR=0, OPOS=0, UBP=1, UAP=1, WOLATE=1, SINIT=1):
    def scope(n):
        if scopes:
            return jax.named_scope(n)
        return contextlib.nullcontext()

    def kernel_body(axT_h, awqkv_h, awo_h, bxT_h, bwq_h, bwkT_h, bwvT_h, bwo_h,
                    out_h,
                    xa_s, xb_s, wqkv_s, wq_s, wo_s, wkv_s,
                    wqT_s, wT_s, woT_s, wkvT_s, qT_s, krep_s, vTb_s, pad_s, sB_s, mB_s, oc_s, oB_s,
                    qTa_s, kA_s, vTa_s, sA_s, mA_s, oA_s, out_s, kmask_s, kvar_s, sems, xsems, osems):

        def cp(src, dst, i):
            return pltpu.make_async_copy(src, dst, sems.at[i])

        def xbcopy(c):
            cols = pl.ds(pl.multiple_of(c * TQ, TQ), TQ)
            return pltpu.make_async_copy(bxT_h.at[:, cols], xb_s.at[:, cols], xsems.at[c])

        c_wq = cp(bwq_h, wq_s, 0)
        c_wk = cp(bwkT_h, wkv_s.at[0], 1)
        c_wv = cp(bwvT_h, wkv_s.at[1], 2)
        c_wob = cp(bwo_h, wo_s.at[1], 3)
        c_wqkv = cp(awqkv_h, wqkv_s, 4)
        c_xa = cp(axT_h, xa_s, 5)
        c_woa = cp(awo_h, wo_s.at[0], 6)

        with scope('Bprep'):
            c_wk.start(priority=PR1)
            c_wv.start(priority=PR1)
            c_wq.start(priority=PR1)
            xbcopy(0).start(priority=PR1)
            if DMAALL:
                for c in range(1, NC):
                    xbcopy(c).start(priority=PR1)
                c_wqkv.start(priority=PR2)
                c_wob.start(priority=PR2)
                c_woa.start(priority=PR2)
                c_xa.start(priority=PR2)
            lane1 = lax.broadcasted_iota(I32, (1, 128), 1)
            for g in range(NG):
                kA_s[g, 0:256, :] = jnp.broadcast_to(
                    jnp.where(lane1 >= 126, 1.0, 0.0), (256, 128)).astype(BF16)
            vTa_s[:, 0:256] = jnp.zeros((D, 256), F32)
            if SINIT:
                sB_s[1] = jnp.zeros((S, TQ), F32)
            mB_s[...] = jnp.zeros((8, TQ), F32)
            oc_s[...] = jnp.zeros((3, 24, TQ), F32)
            lane8 = lax.broadcasted_iota(I32, (8, 128), 1)
            for j in range(7):
                kmask_s[j] = jnp.where((lane8 >= DH * j) & (lane8 < DH * j + DH), I32(-1), I32(0))
            c_wk.wait()
            c_wv.wait()
            wkT = wkv_s[0].astype(F32)
            wvT = wkv_s[1].astype(F32)
            z6 = jnp.zeros((6, D), F32)
            wkvT_s[...] = jnp.concatenate([wkT, z6, wvT, z6], axis=0).astype(BF16)
            c_wq.wait()
            wqT_s[...] = wq_s[...].T

        def b_proj(c, carry):
            row24 = lax.broadcasted_iota(I32, (24, TQ), 0)
            cols = pl.ds(pl.multiple_of(c * TQ, TQ), TQ)
            xbcopy(c).wait()

            if not DMAALL:
                @pl.when(c + 1 < NC)
                def _():
                    xbcopy(c + 1).start()

                @pl.when(c == 1)
                def _():
                    c_wqkv.start()
                    c_wob.start()
                    c_woa.start()
            xT = xb_s[:, cols]
            kvT = jnp.dot(wkvT_s[...], xT, preferred_element_type=F32)
            k = kvT[0:DH]
            kr = jnp.concatenate([k] * 7 + [jnp.zeros((2, TQ), F32)], axis=0).astype(BF16).T
            krows = pl.ds(pl.multiple_of(c * (TQ // 2), TQ // 2), TQ // 2)
            krep_s[krows, :] = pltpu.bitcast(kr, I32)
            if KVAR:
                ki = krep_s[krows, :]
                lane1 = lax.broadcasted_iota(I32, (1, 128), 1)
                for j in range(7):
                    kvar_s[j, krows, :] = ki & jnp.where(
                        (lane1 >= DH * j) & (lane1 < DH * j + DH), I32(-1), I32(0))
            vT = kvT[24:48].astype(BF16).astype(F32)
            for jj in range(4):
                off = 2 * jj
                if off:
                    vv = jnp.concatenate([jnp.zeros((off, TQ), F32), vT[0:24 - off]], axis=0)
                else:
                    vv = vT
                vTb_s[jj, :, cols] = jnp.where(row24 == _lrow(jj), 1.0, vv)
            qT = jnp.dot(wqT_s[...], xT, preferred_element_type=F32) * QSCALE
            qT_s[:, cols] = _pad_group_rows(qT).astype(BF16)
            return carry

        with scope('Bproj'):
            lax.fori_loop(0, NC, b_proj, 0, unroll=UBP)
        if not DMAALL:
            c_xa.start()

        NCH = S // 128

        def b_qk_pre(it):
            h = it % H
            j = h % 7
            if KTAB:
                return kmask_s[j]
            lane = lax.broadcasted_iota(I32, (8, 128), 1)
            return jnp.where((lane >= DH * j) & (lane < DH * j + DH), I32(-1), I32(0))

        def b_qk_chunk(it, c, slot, m, kmask):
            qt = it // H
            g = (it % H) // 7
            w = qT_s[pl.ds(pl.multiple_of(g * 128, 128), 128), pl.ds(pl.multiple_of(qt * TQ, TQ), TQ)]
            if KVAR:
                k = pltpu.bitcast(kvar_s[(it % H) % 7, pl.ds(c * 64, 64), :], BF16)
            else:
                ki = krep_s[pl.ds(c * 64, 64), :].reshape(8, 8, 128) & kmask
                k = pltpu.bitcast(ki.reshape(64, 128), BF16)
            s = jnp.dot(k, w, preferred_element_type=F32)
            sB_s[slot, pl.ds(c * 128, 128), :] = s
            mm = jnp.max(s.reshape(16, 8, TQ), axis=0)
            return mm if m is None else jnp.maximum(m, mm)

        def b_fin_m(m8):
            mB_s[...] = jnp.broadcast_to(jnp.max(m8, axis=0, keepdims=True), (8, TQ))

        def b_pv_chunk(c, slot, jj, m, acc):
            p = jnp.exp2(sB_s[slot, pl.ds(c * 128, 128), :] - m).astype(BF16)
            o = jnp.dot(vTb_s[jj, :, pl.ds(c * 128, 128)], p, preferred_element_type=F32)
            return o if acc is None else acc + o

        NIT = NC * H

        def b_store_unit(iu, outs):
            row8 = lax.broadcasted_iota(I32, (8, TQ), 0)
            qt = iu // 8
            u = iu % 8
            oB_s[pl.ds(pl.multiple_of(u * 72, 8), 72),
                 pl.ds(pl.multiple_of(qt * TQ, TQ), TQ)] = _assemble(outs, row8)

        def b_norm(acc, jj):
            lr = _lrow(jj)
            return acc * (1.0 / acc[lr:lr + 1, :])

        def b_body(i, carry):
            seq = [(st, c) for st in range(UB) for c in range(NCH)]
            mns, ms, accs, kmasks, outs = {}, {}, {}, {}, {}
            for n in range(len(seq) + LAG):
                if n < len(seq):
                    st, c = seq[n]
                    it = i * UB + st
                    if c == 0:
                        kmasks[st] = b_qk_pre(it)
                    mns[st] = b_qk_chunk(it, c, st % 2, mns.get(st), kmasks[st])
                if n >= LAG:
                    st, c = seq[n - LAG]
                    jj = (st - 1) % 4
                    if c == 0:
                        ms[st] = (mB_s[...][0:1, :] if st == 0
                                  else jnp.max(mns[st - 1], axis=0, keepdims=True))
                    accs[st] = b_pv_chunk(c, (st - 1) % 2, jj, ms[st], accs.get(st))
                    if c == NCH - 1:
                        outs[jj] = b_norm(accs[st], jj)
                        if st == 0:
                            iu = jnp.where(i == 0, NIT // 4, i * (UB // 4) - 1)
                            b_store_unit(iu, [oc_s[0], oc_s[1], oc_s[2], outs[3]])
                        elif jj == 3:
                            b_store_unit(i * (UB // 4) + st // 4 - 1, outs)
            for jj in range(3):
                oc_s[jj] = outs[jj]
            b_fin_m(mns[UB - 1])
            return carry

        def a_proj(c, carry):
            cols = pl.ds(pl.multiple_of(c * TQ, TQ), TQ)
            pcols = pl.ds(pl.multiple_of(256 + c * TQ, 256), TQ)
            xT = xa_s[:, cols]
            kT = jnp.dot(wT_s[D:2 * D, :], xT, preferred_element_type=F32)
            kT = _pad_group_rows(kT).astype(BF16)
            for g in range(NG):
                kA_s[g, pcols, :] = kT[128 * g:128 * (g + 1)].T
            qT = jnp.dot(wT_s[0:D, :], xT, preferred_element_type=F32) * QSCALE
            qTa_s[:, cols] = pltpu.bitcast(_pad_group_rows(qT).astype(BF16), I32)
            vT = jnp.dot(wT_s[2 * D:3 * D, :], xT, preferred_element_type=F32)
            vTa_s[:, pcols] = vT.astype(BF16).astype(F32)
            return carry

        with scope('Battn'):
            lax.fori_loop(0, NIT // UB, b_body, 0)
        with scope('Bpost'):
            c_wob.wait()
            c_wqkv.wait()
            c_woa.wait()
            wT_s[...] = wqkv_s[...].T
            if not WOLATE:
                woT_s[0] = wo_s[0].T
                woT_s[1] = wo_s[1].T
            acc = None
            mlast = mB_s[...][0:1, :]
            for c in range(NCH):
                acc = b_pv_chunk(c, 1, 3, mlast, acc)
            b_store_unit(NIT // 4 - 1, [oc_s[0], oc_s[1], oc_s[2], b_norm(acc, 3)])
            if MERGE:
                c_xa.wait()
                a_proj(0, 0)

        with scope('Aproj'):
            if MERGE:
                lax.fori_loop(1, NC, a_proj, 0, unroll=UAP)
            else:
                c_xa.wait()
                lax.fori_loop(0, NC, a_proj, 0, unroll=UAP)

        def a_wts(qt, h):
            r8 = lax.broadcasted_iota(I32, (8, 128), 0)
            g, j = h // 7, h % 7
            q0 = pl.multiple_of(qt * 128, 128)
            lo, hi = 9 * j, 9 * j + 9
            blocks = []
            for b in range(8):
                r0 = 8 * b
                if r0 + 8 <= lo or r0 >= hi:
                    blk = jnp.zeros((8, 128), I32)
                else:
                    blk = qTa_s[pl.ds(64 * g + r0, 8), pl.ds(q0, 128)]
                    if not (r0 >= lo and r0 + 8 <= hi):
                        blk = jnp.where((r8 + r0 >= lo) & (r8 + r0 < hi), blk, I32(0))
                if b == 7:
                    blk = jnp.where(r8 == 7, I32(NEG2), blk)
                blocks.append(blk)
            return pltpu.bitcast(jnp.concatenate(blocks, axis=0), BF16)

        def a_qk_rows(qt, h, slot, hh, r0, r1, w, mm):
            g = h // 7
            q0 = pl.multiple_of(qt * 128, 128)
            s = jnp.dot(kA_s[g, pl.ds(q0 + r0, r1 - r0), :], w, preferred_element_type=F32)
            r64 = lax.broadcasted_iota(I32, (64, 128), 0)
            l64 = lax.broadcasted_iota(I32, (64, 128), 1)
            for a in range(r0, r1, 64):
                blk = s[a - r0:a - r0 + 64]
                if a < 128:
                    blk = jnp.where(r64 + a > l64, blk, NEG)
                elif a >= 256:
                    blk = jnp.where(r64 + (a - 256) <= l64, blk, NEG)
                sA_s[slot, hh, a:a + 64, :] = blk
                mm = blk if mm is None else jnp.maximum(mm, blk)
            return mm

        def a_fin_m(mm, slot, hh):
            mm = jnp.max(mm.reshape(8, 8, 128), axis=0)
            mA_s[slot, hh] = jnp.broadcast_to(jnp.max(mm, axis=0, keepdims=True), (8, 128))

        def a_qk_head(qt, h, slot, hh):
            a_fin_m(a_qk_rows(qt, h, slot, hh, 0, 384, a_wts(qt, h), None), slot, hh)

        def a_pv_tile(qt, h, slot, hh, t, acc):
            r24 = lax.broadcasted_iota(I32, (24, 128), 0)
            q0 = pl.multiple_of(qt * 128 + 128 * t, 128)
            r0 = (DH * h) // 8 * 8
            lr = _lrow(h % 4)
            m = mA_s[slot, hh][0:1, :]
            p = jnp.exp2(sA_s[slot, hh, 128 * t:128 * (t + 1), :] - m).astype(BF16)
            v = jnp.where(r24 == lr, 1.0, vTa_s[r0:r0 + 24, pl.ds(q0, 128)])
            o = jnp.dot(v, p, preferred_element_type=F32)
            return o if acc is None else acc + o

        NQT = S // 128

        def a_qtile(qt, oslot, qq, hook=None):
            row8a = lax.broadcasted_iota(I32, (8, 128), 0)
            for s in range(8):
                slot = s % 2
                if s < 7:
                    nqt, nh0 = qt, (s + 1) * 4
                else:
                    nqt, nh0 = jnp.minimum(qt + 1, NQT - 1), 0
                ws = [a_wts(nqt, nh0 + hh) for hh in range(4)]
                mms = [a_qk_rows(nqt, nh0 + hh, 1 - slot, hh, 0, CUT, ws[hh], None) for hh in range(4)]
                accs = [a_pv_tile(qt, s * 4 + hh, slot, hh, 0, None) for hh in range(4)]
                mms = [a_qk_rows(nqt, nh0 + hh, 1 - slot, hh, CUT, 384, ws[hh], mms[hh]) for hh in range(4)]
                for t in (1, 2):
                    accs = [a_pv_tile(qt, s * 4 + hh, slot, hh, t, accs[hh]) for hh in range(4)]
                for hh in range(4):
                    a_fin_m(mms[hh], 1 - slot, hh)
                outs = [accs[hh] * (1.0 / accs[hh][_lrow(hh):_lrow(hh) + 1, :]) for hh in range(4)]
                oA_s[oslot, pl.ds(72 * s, 72), pl.ds(qq * 128, 128)] = _assemble(outs, row8a)
                if hook is not None:
                    hook(s)

        TF = 256
        NT_ = S // TF

        def fcopy(t, part):
            rows = pl.ds(pl.multiple_of(t * TF, TF), TF)
            cols = pl.ds(0, 640) if part == 0 else pl.ds(640, 512)
            return pltpu.make_async_copy(out_s.at[rows, cols], out_h.at[rows, cols], osems.at[t, part])

        def out_proj(t):
            rows = pl.ds(pl.multiple_of(t * TF, TF), TF)
            ob = oB_s[:, rows].astype(BF16)
            oa = oA_s[t % 2].astype(BF16)
            for i in range(9):
                if i < 4:
                    r = jnp.dot(woT_s[0, 128 * i:128 * (i + 1), :], oa, preferred_element_type=F32)
                elif i == 4:
                    ra = jnp.dot(woT_s[0, 512:576, :], oa, preferred_element_type=F32)
                    rb = jnp.dot(woT_s[1, 0:64, :], ob, preferred_element_type=F32)
                    r = jnp.concatenate([ra, rb], axis=0)
                else:
                    r0 = 64 + 128 * (i - 5)
                    r = jnp.dot(woT_s[1, r0:r0 + 128, :], ob, preferred_element_type=F32)
                out_s[rows, 128 * i:128 * (i + 1)] = r.astype(BF16).T
                if i == 4:
                    fcopy(t, 0).start()
            fcopy(t, 1).start()

        def attn_tile(t):
            for qq in range(2):
                a_qtile(2 * t + qq, t % 2, qq)

        def f_tile(t, carry):
            if OPOS == 0:
                out_proj(t - 1)
                attn_tile(t)
            elif OPOS == 1:
                a_qtile(2 * t, t % 2, 0)
                out_proj(t - 1)
                a_qtile(2 * t + 1, t % 2, 1)
            elif OPOS == 2:
                attn_tile(t)
                out_proj(t - 1)
            else:
                a_qtile(2 * t, t % 2, 0, lambda s_: out_proj(t - 1) if s_ == OPOS - 3 else None)
                a_qtile(2 * t + 1, t % 2, 1)
            return carry

        with scope('Aattn'):
            if WOLATE:
                woT_s[0] = wo_s[0].T
                woT_s[1] = wo_s[1].T
            for hh in range(4):
                a_qk_head(0, hh, 0, hh)
            attn_tile(0)
            lax.fori_loop(1, NT_, f_tile, 0)
            out_proj(NT_ - 1)
        for t in range(NT_):
            fcopy(t, 0).wait()
            fcopy(t, 1).wait()

    return kernel_body


FLAGSETS = {
    1: {'XLA_TPU_EVENLY_DISTRIBUTE_CRITICAL_NODES': True},
    2: {'XLA_TPU_EVENLY_DISTRIBUTE_CRITICAL_NODES': True, 'XLA_TPU_RESCHEDULE_DMA_DONES': True},
    3: {'XLA_TPU_EVENLY_DISTRIBUTE_CRITICAL_NODES': True, 'XLA_TPU_ENABLE_LLO_SMALL_LOOP_FLATTENING': True},
    4: {'XLA_TPU_EVENLY_DISTRIBUTE_CRITICAL_NODES': True, 'XLA_TPU_MAX_INSTS_TO_PREDICATE': 65536},
}


def build(name="k8", FLAGS=1, PAD1=0, PAD2=0, **kw):
    scratch = [
        pltpu.VMEM((D, S), BF16),
        pltpu.VMEM((D, S), BF16),
        pltpu.VMEM((D, 3 * D), BF16),
        pltpu.VMEM((D, D), BF16),
        pltpu.VMEM((2, D, D), BF16),
        pltpu.VMEM((2, DH, D), BF16),
        pltpu.VMEM((D, D), BF16),
        pltpu.VMEM((3 * D, D), BF16),
        pltpu.VMEM((2, D, D), BF16),
        pltpu.VMEM((48, D), BF16),
        pltpu.VMEM((640, S), BF16),
        pltpu.VMEM((S // 2, 128), I32),
        pltpu.VMEM((4, 24, S), F32),
        pltpu.VMEM((8 + 8 * PAD1, 128), F32),
        pltpu.VMEM((2, S + 8 * PAD2, TQ), F32),
        pltpu.VMEM((8, TQ), F32),
        pltpu.VMEM((3, 24, TQ), F32),
        pltpu.VMEM((D, S + TQ), F32),
        pltpu.VMEM((320, S), I32),
        pltpu.VMEM((NG, S + 256, 128), BF16),
        pltpu.VMEM((D, S + 256), F32),
        pltpu.VMEM((2, 4, 384, 128), F32),
        pltpu.VMEM((2, 4, 8, 128), F32),
        pltpu.VMEM((2, D, 256), F32),
        pltpu.VMEM((S, 2 * D), BF16),
        pltpu.VMEM((7, 8, 128), I32),
        pltpu.VMEM((7, S // 2, 128), I32),
        pltpu.SemaphoreType.DMA((7,)),
        pltpu.SemaphoreType.DMA((NC,)),
        pltpu.SemaphoreType.DMA((8, 2)),
    ]
    any_spec = pl.BlockSpec(memory_space=pl.ANY)
    return pl.pallas_call(
        make_body(**kw),
        out_shape=jax.ShapeDtypeStruct((S, 2 * D), BF16),
        in_specs=[any_spec] * 8,
        out_specs=any_spec,
        scratch_shapes=scratch,
        name=name,
        compiler_params=pltpu.CompilerParams(vmem_limit_bytes=110 * 1024 * 1024,
                                             flags=(FLAGSETS[FLAGS] if FLAGS else None)),
    )


@jax.jit
def pallas_concat_heads__sliding_block__grouped_kv_mqa__prompt_kernel(
    A_x: jax.Array,
    A_wqkv: jax.Array,
    A_wo: jax.Array,
    B_x: jax.Array,
    B_wq: jax.Array,
    B_wk: jax.Array,
    B_wv: jax.Array,
    B_wo: jax.Array,
):
    out = build()(A_x[0].T, A_wqkv, A_wo, B_x[0].T, B_wq, B_wk.T, B_wv.T, B_wo)
    return out.reshape(1, S, 2 * D)
```

```python
import jax
import jax.numpy as jnp
import numpy as np
from jax import lax
from jax.experimental import pallas as pl
from jax.experimental.pallas import tpu as pltpu

S = 2048
D = 576
H = 32
DH = 18
WIN = 256
NG = 5
TQ = 512
NC = S // TQ
KCH = S // 128
NIT = NC * H
UB = 8
TF = 256
NF = S // TF
NEG = -1e30
QSCALE = float(DH ** -0.5 * np.log2(np.e))
F32 = jnp.float32
BF16 = jnp.bfloat16
I32 = jnp.int32

_NEG_BITS = int(np.array([NEG], dtype=np.float32).view(np.uint32)[0] >> 16)
NEG2 = int(np.array([(_NEG_BITS << 16) | _NEG_BITS], dtype=np.uint32).view(np.int32)[0])


def _pad_group_rows(wt):
    n = wt.shape[1]
    parts = []
    for g in range(NG):
        lo = 126 * g
        hi = min(lo + 126, D)
        parts.append(wt[lo:hi])
        parts.append(jnp.zeros((128 - (hi - lo), n), wt.dtype))
    return jnp.concatenate(parts, axis=0)


def _lrow(jj):
    return 23 if jj < 3 else 0


def _normalise(o, jj):
    lr = _lrow(jj)
    return o * (1.0 / o[lr:lr + 1, :])


def _assemble(o):
    row8 = lax.broadcasted_iota(I32, (8, o[0].shape[1]), 0)

    def sel(k, a, b):
        return jnp.where(row8 < k, a, b)

    return jnp.concatenate([
        o[0][0:8], o[0][8:16], sel(2, o[0][16:24], o[1][0:8]),
        o[1][8:16], sel(4, o[1][16:24], o[2][0:8]),
        o[2][8:16], sel(6, o[2][16:24], o[3][0:8]),
        o[3][8:16], o[3][16:24]], axis=0)


def _kernel(axT_h, awqkv_h, awo_h, bxT_h, bwq_h, bwkT_h, bwvT_h, bwo_h, out_h,
            xa_s, xb_s, wqkv_s, wq_s, wo_s, wkv_s, wqT_s, wT_s, woT_s, wkvT_s,
            qTb_s, krep_s, vTb_s, sB_s, mB_s, oc_s, oB_s,
            qTa_s, kA_s, vTa_s, sA_s, mA_s, oA_s, out_s,
            sems, xsems, osems):
    def cp(src, dst, i):
        return pltpu.make_async_copy(src, dst, sems.at[i])

    def xb_copy(c):
        cols = pl.ds(pl.multiple_of(c * TQ, TQ), TQ)
        return pltpu.make_async_copy(bxT_h.at[:, cols], xb_s.at[:, cols], xsems.at[c])

    def out_copy(t, part):
        rows = pl.ds(pl.multiple_of(t * TF, TF), TF)
        cols = pl.ds(0, 640) if part == 0 else pl.ds(640, 512)
        return pltpu.make_async_copy(out_s.at[rows, cols], out_h.at[rows, cols], osems.at[t, part])

    c_wq = cp(bwq_h, wq_s, 0)
    c_wk = cp(bwkT_h, wkv_s.at[0], 1)
    c_wv = cp(bwvT_h, wkv_s.at[1], 2)
    c_wob = cp(bwo_h, wo_s.at[1], 3)
    c_wqkv = cp(awqkv_h, wqkv_s, 4)
    c_xa = cp(axT_h, xa_s, 5)
    c_woa = cp(awo_h, wo_s.at[0], 6)

    c_wk.start()
    c_wv.start()
    c_wq.start()
    lane1 = lax.broadcasted_iota(I32, (1, 128), 1)
    for g in range(NG):
        kA_s[g, 0:WIN, :] = jnp.broadcast_to(
            jnp.where(lane1 >= 126, 1.0, 0.0), (WIN, 128)).astype(BF16)
    vTa_s[:, 0:WIN] = jnp.zeros((D, WIN), F32)
    sB_s[1] = jnp.zeros((S, TQ), F32)
    mB_s[...] = jnp.zeros((8, TQ), F32)
    oc_s[...] = jnp.zeros((3, 24, TQ), F32)
    c_wk.wait()
    c_wv.wait()
    for c in range(NC):
        xb_copy(c).start()
    c_wqkv.start(priority=1)
    c_xa.start(priority=1)
    c_wob.start(priority=1)
    c_woa.start(priority=1)
    z6 = jnp.zeros((6, D), F32)
    wkvT_s[...] = jnp.concatenate(
        [wkv_s[0].astype(F32), z6, wkv_s[1].astype(F32), z6], axis=0).astype(BF16)
    c_wq.wait()
    wqT_s[...] = wq_s[...].T

    def b_proj(c, carry):
        row24 = lax.broadcasted_iota(I32, (24, TQ), 0)
        cols = pl.ds(pl.multiple_of(c * TQ, TQ), TQ)
        xb_copy(c).wait()
        xT = xb_s[:, cols]
        kvT = jnp.dot(wkvT_s[...], xT, preferred_element_type=F32)
        k = kvT[0:DH]
        kr = jnp.concatenate([k] * 7 + [jnp.zeros((2, TQ), F32)], axis=0).astype(BF16).T
        krep_s[pl.ds(pl.multiple_of(c * (TQ // 2), TQ // 2), TQ // 2), :] = pltpu.bitcast(kr, I32)
        vT = kvT[24:48].astype(BF16).astype(F32)
        for jj in range(4):
            off = 2 * jj
            vv = (jnp.concatenate([jnp.zeros((off, TQ), F32), vT[0:24 - off]], axis=0)
                  if off else vT)
            vTb_s[jj, :, cols] = jnp.where(row24 == _lrow(jj), 1.0, vv)
        qT = jnp.dot(wqT_s[...], xT, preferred_element_type=F32) * QSCALE
        qTb_s[:, cols] = _pad_group_rows(qT).astype(BF16)
        return carry

    lax.fori_loop(0, NC, b_proj, 0)

    def b_kmask(it):
        j = (it % H) % 7
        lane = lax.broadcasted_iota(I32, (8, 128), 1)
        return jnp.where((lane >= DH * j) & (lane < DH * j + DH), I32(-1), I32(0))

    def b_scores(it, c, slot, m, kmask):
        qt = it // H
        g = (it % H) // 7
        w = qTb_s[pl.ds(pl.multiple_of(g * 128, 128), 128), pl.ds(pl.multiple_of(qt * TQ, TQ), TQ)]
        ki = krep_s[pl.ds(c * 64, 64), :].reshape(8, 8, 128) & kmask
        k = pltpu.bitcast(ki.reshape(64, 128), BF16)
        s = jnp.dot(k, w, preferred_element_type=F32)
        sB_s[slot, pl.ds(c * 128, 128), :] = s
        mm = jnp.max(s.reshape(16, 8, TQ), axis=0)
        return mm if m is None else jnp.maximum(m, mm)

    def b_pv(c, slot, jj, m, acc):
        p = jnp.exp2(sB_s[slot, pl.ds(c * 128, 128), :] - m).astype(BF16)
        o = jnp.dot(vTb_s[jj, :, pl.ds(c * 128, 128)], p, preferred_element_type=F32)
        return o if acc is None else acc + o

    def b_store_unit(iu, outs):
        oB_s[pl.ds(pl.multiple_of((iu % 8) * 72, 8), 72),
             pl.ds(pl.multiple_of((iu // 8) * TQ, TQ), TQ)] = _assemble(outs)

    def b_body(i, carry):
        seq = [(st, c) for st in range(UB) for c in range(KCH)]
        mx, ms, accs, kmasks, outs = {}, {}, {}, {}, {}
        for n in range(len(seq) + 1):
            if n < len(seq):
                st, c = seq[n]
                it = i * UB + st
                if c == 0:
                    kmasks[st] = b_kmask(it)
                mx[st] = b_scores(it, c, st % 2, mx.get(st), kmasks[st])
            if n >= 1:
                st, c = seq[n - 1]
                jj = (st - 1) % 4
                if c == 0:
                    ms[st] = (mB_s[...][0:1, :] if st == 0
                              else jnp.max(mx[st - 1], axis=0, keepdims=True))
                accs[st] = b_pv(c, (st - 1) % 2, jj, ms[st], accs.get(st))
                if c == KCH - 1:
                    outs[jj] = _normalise(accs[st], jj)
                    if st == 0:
                        iu = jnp.where(i == 0, NIT // 4, i * (UB // 4) - 1)
                        b_store_unit(iu, [oc_s[0], oc_s[1], oc_s[2], outs[3]])
                    elif jj == 3:
                        b_store_unit(i * (UB // 4) + st // 4 - 1, outs)
        for jj in range(3):
            oc_s[jj] = outs[jj]
        mB_s[...] = jnp.broadcast_to(jnp.max(mx[UB - 1], axis=0, keepdims=True), (8, TQ))
        return carry

    lax.fori_loop(0, NIT // UB, b_body, 0)

    def a_cols(c):
        return (pl.ds(pl.multiple_of(c * TQ, TQ), TQ),
                pl.ds(pl.multiple_of(WIN + c * TQ, WIN), TQ))

    def a_proj_k(c):
        cols, pcols = a_cols(c)
        kT = jnp.dot(wT_s[D:2 * D, :], xa_s[:, cols], preferred_element_type=F32)
        kT = _pad_group_rows(kT).astype(BF16)
        for g in range(NG):
            kA_s[g, pcols, :] = kT[128 * g:128 * (g + 1)].T

    def a_proj_q(c):
        cols, _ = a_cols(c)
        qT = jnp.dot(wT_s[0:D, :], xa_s[:, cols], preferred_element_type=F32) * QSCALE
        qTa_s[:, cols] = pltpu.bitcast(_pad_group_rows(qT).astype(BF16), I32)

    def a_proj_v(c):
        cols, pcols = a_cols(c)
        vT = jnp.dot(wT_s[2 * D:3 * D, :], xa_s[:, cols], preferred_element_type=F32)
        vTa_s[:, pcols] = vT.astype(BF16).astype(F32)

    def a_proj(c, carry):
        a_proj_k(c)
        a_proj_q(c)
        a_proj_v(c)
        return carry

    c_wqkv.wait()
    c_xa.wait()
    m_last = mB_s[...][0:1, :]
    acc = None
    wT_s[2 * D:3 * D, :] = wqkv_s[:, 2 * D:3 * D].T
    a_proj_v(0)
    for c in range(0, 5):
        acc = b_pv(c, 1, 3, m_last, acc)
    wT_s[0:640, :] = wqkv_s[:, 0:640].T
    a_proj_q(0)
    for c in range(5, 11):
        acc = b_pv(c, 1, 3, m_last, acc)
    wT_s[640:2 * D, :] = wqkv_s[:, 640:2 * D].T
    a_proj_k(0)
    for c in range(11, KCH):
        acc = b_pv(c, 1, 3, m_last, acc)
    b_store_unit(NIT // 4 - 1, [oc_s[0], oc_s[1], oc_s[2], _normalise(acc, 3)])
    lax.fori_loop(1, NC, a_proj, 0)

    def a_weights(qt, h):
        r8 = lax.broadcasted_iota(I32, (8, 128), 0)
        g, j = h // 7, h % 7
        q0 = pl.multiple_of(qt * 128, 128)
        lo, hi = 9 * j, 9 * j + 9
        blocks = []
        for b in range(8):
            r0 = 8 * b
            if r0 + 8 <= lo or r0 >= hi:
                blk = jnp.zeros((8, 128), I32)
            else:
                blk = qTa_s[pl.ds(64 * g + r0, 8), pl.ds(q0, 128)]
                if not (r0 >= lo and r0 + 8 <= hi):
                    blk = jnp.where((r8 + r0 >= lo) & (r8 + r0 < hi), blk, I32(0))
            if b == 7:
                blk = jnp.where(r8 == 7, I32(NEG2), blk)
            blocks.append(blk)
        return pltpu.bitcast(jnp.concatenate(blocks, axis=0), BF16)

    def a_scores(qt, h, slot, hh, r0, r1, w, mm):
        q0 = pl.multiple_of(qt * 128, 128)
        s = jnp.dot(kA_s[h // 7, pl.ds(q0 + r0, r1 - r0), :], w, preferred_element_type=F32)
        r64 = lax.broadcasted_iota(I32, (64, 128), 0)
        l64 = lax.broadcasted_iota(I32, (64, 128), 1)
        for a in range(r0, r1, 64):
            blk = s[a - r0:a - r0 + 64]
            if a < 128:
                blk = jnp.where(r64 + a > l64, blk, NEG)
            elif a >= 256:
                blk = jnp.where(r64 + (a - 256) <= l64, blk, NEG)
            sA_s[slot, hh, a:a + 64, :] = blk
            mm = blk if mm is None else jnp.maximum(mm, blk)
        return mm

    def a_store_max(mm, slot, hh):
        mm = jnp.max(mm.reshape(8, 8, 128), axis=0)
        mA_s[slot, hh] = jnp.broadcast_to(jnp.max(mm, axis=0, keepdims=True), (8, 128))

    def a_pv(qt, h, slot, hh, t, acc):
        r24 = lax.broadcasted_iota(I32, (24, 128), 0)
        k0 = pl.multiple_of(qt * 128 + 128 * t, 128)
        r0 = (DH * h) // 8 * 8
        m = mA_s[slot, hh][0:1, :]
        p = jnp.exp2(sA_s[slot, hh, 128 * t:128 * (t + 1), :] - m).astype(BF16)
        v = jnp.where(r24 == _lrow(h % 4), 1.0, vTa_s[r0:r0 + 24, pl.ds(k0, 128)])
        o = jnp.dot(v, p, preferred_element_type=F32)
        return o if acc is None else acc + o

    def a_qtile(qt, oslot, qq):
        for s in range(8):
            slot = s % 2
            if s < 7:
                nqt, nh0 = qt, (s + 1) * 4
            else:
                nqt, nh0 = jnp.minimum(qt + 1, S // 128 - 1), 0
            hs = range(4)
            ws = [a_weights(nqt, nh0 + hh) for hh in hs]
            mms = [a_scores(nqt, nh0 + hh, 1 - slot, hh, 0, 256, ws[hh], None) for hh in hs]
            accs = [a_pv(qt, s * 4 + hh, slot, hh, 0, None) for hh in hs]
            mms = [a_scores(nqt, nh0 + hh, 1 - slot, hh, 256, 384, ws[hh], mms[hh]) for hh in hs]
            for t in (1, 2):
                accs = [a_pv(qt, s * 4 + hh, slot, hh, t, accs[hh]) for hh in hs]
            for hh in hs:
                a_store_max(mms[hh], 1 - slot, hh)
            oA_s[oslot, pl.ds(72 * s, 72), pl.ds(qq * 128, 128)] = _assemble(
                [_normalise(accs[hh], hh) for hh in hs])

    def attn_tile(t):
        for qq in range(2):
            a_qtile(2 * t + qq, t % 2, qq)

    def out_proj(t):
        rows = pl.ds(pl.multiple_of(t * TF, TF), TF)
        ob = oB_s[:, rows].astype(BF16)
        oa = oA_s[t % 2].astype(BF16)
        for i in range(9):
            if i < 4:
                r = jnp.dot(woT_s[0, 128 * i:128 * (i + 1), :], oa, preferred_element_type=F32)
            elif i == 4:
                ra = jnp.dot(woT_s[0, 512:576, :], oa, preferred_element_type=F32)
                rb = jnp.dot(woT_s[1, 0:64, :], ob, preferred_element_type=F32)
                r = jnp.concatenate([ra, rb], axis=0)
            else:
                r0 = 64 + 128 * (i - 5)
                r = jnp.dot(woT_s[1, r0:r0 + 128, :], ob, preferred_element_type=F32)
            out_s[rows, 128 * i:128 * (i + 1)] = r.astype(BF16).T
            if i == 4:
                out_copy(t, 0).start()
        out_copy(t, 1).start()

    def tile_body(t, carry):
        out_proj(t - 1)
        attn_tile(t)
        return carry

    c_wob.wait()
    c_woa.wait()
    woT_s[0] = wo_s[0].T
    woT_s[1] = wo_s[1].T
    for hh in range(4):
        a_store_max(a_scores(0, hh, 0, hh, 0, 384, a_weights(0, hh), None), 0, hh)
    attn_tile(0)
    lax.fori_loop(1, NF, tile_body, 0)
    out_proj(NF - 1)
    for t in range(NF):
        out_copy(t, 0).wait()
        out_copy(t, 1).wait()


def _build():
    scratch = [
        pltpu.VMEM((D, S), BF16),
        pltpu.VMEM((D, S), BF16),
        pltpu.VMEM((D, 3 * D), BF16),
        pltpu.VMEM((D, D), BF16),
        pltpu.VMEM((2, D, D), BF16),
        pltpu.VMEM((2, DH, D), BF16),
        pltpu.VMEM((D, D), BF16),
        pltpu.VMEM((3 * D, D), BF16),
        pltpu.VMEM((2, D, D), BF16),
        pltpu.VMEM((48, D), BF16),
        pltpu.VMEM((640, S), BF16),
        pltpu.VMEM((S // 2, 128), I32),
        pltpu.VMEM((4, 24, S), F32),
        pltpu.VMEM((2, S, TQ), F32),
        pltpu.VMEM((8, TQ), F32),
        pltpu.VMEM((3, 24, TQ), F32),
        pltpu.VMEM((D, S + TQ), F32),
        pltpu.VMEM((320, S), I32),
        pltpu.VMEM((NG, S + WIN, 128), BF16),
        pltpu.VMEM((D, S + WIN), F32),
        pltpu.VMEM((2, 4, 384, 128), F32),
        pltpu.VMEM((2, 4, 8, 128), F32),
        pltpu.VMEM((2, D, TF), F32),
        pltpu.VMEM((S, 2 * D), BF16),
        pltpu.SemaphoreType.DMA((7,)),
        pltpu.SemaphoreType.DMA((NC,)),
        pltpu.SemaphoreType.DMA((NF, 2)),
    ]
    any_spec = pl.BlockSpec(memory_space=pl.ANY)
    return pl.pallas_call(
        _kernel,
        out_shape=jax.ShapeDtypeStruct((S, 2 * D), BF16),
        in_specs=[any_spec] * 8,
        out_specs=any_spec,
        scratch_shapes=scratch,
        name="concat_heads_window_mqa",
        compiler_params=pltpu.CompilerParams(
            vmem_limit_bytes=100 * 1024 * 1024,
            flags={"XLA_TPU_EVENLY_DISTRIBUTE_CRITICAL_NODES": True},
        ),
    )


@jax.jit
def pallas_concat_heads__sliding_block__grouped_kv_mqa__prompt_kernel(
    A_x: jax.Array,
    A_wqkv: jax.Array,
    A_wo: jax.Array,
    B_x: jax.Array,
    B_wq: jax.Array,
    B_wk: jax.Array,
    B_wv: jax.Array,
    B_wo: jax.Array,
):
    out = _build()(A_x[0].T, A_wqkv, A_wo, B_x[0].T, B_wq, B_wk.T, B_wv.T, B_wo)
    return out.reshape(1, S, 2 * D)
```

```python
import jax
import jax.numpy as jnp
import numpy as np
from jax import lax
from jax.experimental import pallas as pl
from jax.experimental.pallas import tpu as pltpu

S = 2048
D = 576
H = 32
DH = 18
HB = 7
HA = 6
NGA = 6
TQ = 512
NC = S // TQ
KCH = S // 128
NIT = NC * H
UB = 8
TF = 256
NF = S // TF
NEG = -1e30
QSCALE = float(DH ** -0.5 * np.log2(np.e))
F32 = jnp.float32
BF16 = jnp.bfloat16
I32 = jnp.int32


def _pad_group_rows(wt, hpg):
    n = wt.shape[1]
    parts = []
    for lo in range(0, D, hpg * DH):
        hi = min(lo + hpg * DH, D)
        parts.append(wt[lo:hi])
        parts.append(jnp.zeros((128 - (hi - lo), n), wt.dtype))
    return jnp.concatenate(parts, axis=0)


def _lrow(jj):
    return 23 if jj < 3 else 0


def _normalise(o, jj):
    lr = _lrow(jj)
    return o * (1.0 / o[lr:lr + 1, :])


def _assemble(o):
    row8 = lax.broadcasted_iota(I32, (8, o[0].shape[1]), 0)

    def sel(k, a, b):
        return jnp.where(row8 < k, a, b)

    return jnp.concatenate([
        o[0][0:8], o[0][8:16], sel(2, o[0][16:24], o[1][0:8]),
        o[1][8:16], sel(4, o[1][16:24], o[2][0:8]),
        o[2][8:16], sel(6, o[2][16:24], o[3][0:8]),
        o[3][8:16], o[3][16:24]], axis=0)


def _kernel(axT_h, awqkv_h, awo_h, bxT_h, bwq_h, bwkT_h, bwvT_h, bwo_h, out_h,
            xa_s, xb_s, wqkv_s, wq_s, wo_s, wkv_s, wqT_s, wT_s, woT_s, wkvT_s,
            qTb_s, krep_s, vTb_s, sB_s, mB_s, oc_s, oB_s,
            qTa_s, kA_s, vTa_s, sA_s, mA_s, sE_s, mE_s, oA_s, out_s,
            sems, xsems, osems):
    def cp(src, dst, i):
        return pltpu.make_async_copy(src, dst, sems.at[i])

    def xb_copy(c):
        cols = pl.ds(pl.multiple_of(c * TQ, TQ), TQ)
        return pltpu.make_async_copy(bxT_h.at[:, cols], xb_s.at[:, cols], xsems.at[c])

    def out_copy(t, part):
        rows = pl.ds(pl.multiple_of(t * TF, TF), TF)
        cols = pl.ds(0, 640) if part == 0 else pl.ds(640, 512)
        return pltpu.make_async_copy(out_s.at[rows, cols], out_h.at[rows, cols], osems.at[t, part])

    c_wq = cp(bwq_h, wq_s, 0)
    c_wk = cp(bwkT_h, wkv_s.at[0], 1)
    c_wv = cp(bwvT_h, wkv_s.at[1], 2)
    c_wob = cp(bwo_h, wo_s.at[1], 3)
    c_wqkv = cp(awqkv_h, wqkv_s, 4)
    c_xa = cp(axT_h, xa_s, 5)
    c_woa = cp(awo_h, wo_s.at[0], 6)

    c_wk.start()
    c_wv.start()
    c_wq.start()
    sB_s[1] = jnp.zeros((S, TQ), F32)
    mB_s[...] = jnp.zeros((8, TQ), F32)
    oc_s[...] = jnp.zeros((3, 24, TQ), F32)
    c_wk.wait()
    c_wv.wait()
    for c in range(NC):
        xb_copy(c).start()
    c_wqkv.start(priority=1)
    c_xa.start(priority=1)
    c_wob.start(priority=1)
    c_woa.start(priority=1)
    z6 = jnp.zeros((6, D), F32)
    wkvT_s[...] = jnp.concatenate(
        [wkv_s[0].astype(F32), z6, wkv_s[1].astype(F32), z6], axis=0).astype(BF16)
    c_wq.wait()
    wqT_s[...] = wq_s[...].T

    def b_proj(c, carry):
        row24 = lax.broadcasted_iota(I32, (24, TQ), 0)
        cols = pl.ds(pl.multiple_of(c * TQ, TQ), TQ)
        xb_copy(c).wait()
        xT = xb_s[:, cols]
        kvT = jnp.dot(wkvT_s[...], xT, preferred_element_type=F32)
        k = kvT[0:DH]
        kr = jnp.concatenate([k] * 7 + [jnp.zeros((2, TQ), F32)], axis=0).astype(BF16).T
        krep_s[pl.ds(pl.multiple_of(c * (TQ // 2), TQ // 2), TQ // 2), :] = pltpu.bitcast(kr, I32)
        vT = kvT[24:48].astype(BF16).astype(F32)
        for jj in range(4):
            off = 2 * jj
            vv = (jnp.concatenate([jnp.zeros((off, TQ), F32), vT[0:24 - off]], axis=0)
                  if off else vT)
            vTb_s[jj, :, cols] = jnp.where(row24 == _lrow(jj), 1.0, vv)
        qT = jnp.dot(wqT_s[...], xT, preferred_element_type=F32) * QSCALE
        qTb_s[:, cols] = _pad_group_rows(qT, HB).astype(BF16)
        return carry

    lax.fori_loop(0, NC, b_proj, 0)

    def b_kmask(it):
        j = (it % H) % 7
        lane = lax.broadcasted_iota(I32, (8, 128), 1)
        return jnp.where((lane >= DH * j) & (lane < DH * j + DH), I32(-1), I32(0))

    def b_scores(it, c, slot, m, kmask):
        qt = it // H
        g = (it % H) // 7
        w = qTb_s[pl.ds(pl.multiple_of(g * 128, 128), 128), pl.ds(pl.multiple_of(qt * TQ, TQ), TQ)]
        ki = krep_s[pl.ds(c * 64, 64), :].reshape(8, 8, 128) & kmask
        k = pltpu.bitcast(ki.reshape(64, 128), BF16)
        s = jnp.dot(k, w, preferred_element_type=F32)
        sB_s[slot, pl.ds(c * 128, 128), :] = s
        mm = jnp.max(s.reshape(16, 8, TQ), axis=0)
        return mm if m is None else jnp.maximum(m, mm)

    def b_pv(c, slot, jj, m, acc):
        p = jnp.exp2(sB_s[slot, pl.ds(c * 128, 128), :] - m).astype(BF16)
        o = jnp.dot(vTb_s[jj, :, pl.ds(c * 128, 128)], p, preferred_element_type=F32)
        return o if acc is None else acc + o

    def b_store_unit(iu, outs):
        oB_s[pl.ds(pl.multiple_of((iu % 8) * 72, 8), 72),
             pl.ds(pl.multiple_of((iu // 8) * TQ, TQ), TQ)] = _assemble(outs)

    def b_body(i, carry):
        seq = [(st, c) for st in range(UB) for c in range(KCH)]
        mx, ms, accs, kmasks, outs = {}, {}, {}, {}, {}
        for n in range(len(seq) + 1):
            if n < len(seq):
                st, c = seq[n]
                it = i * UB + st
                if c == 0:
                    kmasks[st] = b_kmask(it)
                mx[st] = b_scores(it, c, st % 2, mx.get(st), kmasks[st])
            if n >= 1:
                st, c = seq[n - 1]
                jj = (st - 1) % 4
                if c == 0:
                    ms[st] = (mB_s[...][0:1, :] if st == 0
                              else jnp.max(mx[st - 1], axis=0, keepdims=True))
                accs[st] = b_pv(c, (st - 1) % 2, jj, ms[st], accs.get(st))
                if c == KCH - 1:
                    outs[jj] = _normalise(accs[st], jj)
                    if st == 0:
                        iu = jnp.where(i == 0, NIT // 4, i * (UB // 4) - 1)
                        b_store_unit(iu, [oc_s[0], oc_s[1], oc_s[2], outs[3]])
                    elif jj == 3:
                        b_store_unit(i * (UB // 4) + st // 4 - 1, outs)
        for jj in range(3):
            oc_s[jj] = outs[jj]
        mB_s[...] = jnp.broadcast_to(jnp.max(mx[UB - 1], axis=0, keepdims=True), (8, TQ))
        return carry

    lax.fori_loop(0, NIT // UB, b_body, 0)

    def a_cols(c):
        return pl.ds(pl.multiple_of(c * TQ, TQ), TQ)

    def a_proj_k(c):
        cols = a_cols(c)
        kT = jnp.dot(wT_s[D:2 * D, :], xa_s[:, cols], preferred_element_type=F32)
        kT = _pad_group_rows(kT, HA)
        for g in range(NGA):
            n = pltpu.bitcast(kT[128 * g:128 * (g + 1)].astype(BF16).T, I32).reshape(TQ // 16, 1, 8, 128)
            even = lax.bitcast_convert_type(n << 16, F32)
            odd = lax.bitcast_convert_type(n & I32(-65536), F32)
            kA_s[g, cols, :] = jnp.concatenate([even, odd], axis=1).reshape(TQ, 128).astype(BF16)

    def a_proj_q(c):
        cols = a_cols(c)
        qT = jnp.dot(wT_s[0:D, :], xa_s[:, cols], preferred_element_type=F32) * QSCALE
        qTa_s[:, cols] = pltpu.bitcast(_pad_group_rows(qT, HA).astype(BF16), I32)

    def a_proj_v(c):
        cols = a_cols(c)
        vT = jnp.dot(wT_s[2 * D:3 * D, :], xa_s[:, cols], preferred_element_type=F32)
        vTa_s[:, cols] = vT.astype(BF16).astype(F32)

    def a_proj(c, carry):
        a_proj_k(c)
        a_proj_q(c)
        a_proj_v(c)
        return carry

    c_wqkv.wait()
    c_xa.wait()
    m_last = mB_s[...][0:1, :]
    acc = None
    wT_s[2 * D:3 * D, :] = wqkv_s[:, 2 * D:3 * D].T
    a_proj_v(0)
    for c in range(0, 5):
        acc = b_pv(c, 1, 3, m_last, acc)
    wT_s[0:640, :] = wqkv_s[:, 0:640].T
    a_proj_q(0)
    for c in range(5, 11):
        acc = b_pv(c, 1, 3, m_last, acc)
    wT_s[640:2 * D, :] = wqkv_s[:, 640:2 * D].T
    a_proj_k(0)
    for c in range(11, KCH):
        acc = b_pv(c, 1, 3, m_last, acc)
    b_store_unit(NIT // 4 - 1, [oc_s[0], oc_s[1], oc_s[2], _normalise(acc, 3)])
    lax.fori_loop(1, NC, a_proj, 0)

    def a_weights(qt, pr):
        g, ja = (2 * pr) // HA, (2 * pr) % HA
        jb = ja + 1
        q0 = pl.multiple_of(qt * 128, 128)
        r8 = lax.broadcasted_iota(I32, (8, 128), 0)
        lo = lax.broadcasted_iota(I32, (8, 128), 1) < 64
        wl, wu = [], []
        for r0 in range(0, 64, 8):
            if r0 + 8 <= 9 * ja or r0 >= 9 * jb + 9:
                wl.append(jnp.zeros((8, 128), I32))
                wu.append(jnp.zeros((8, 128), I32))
                continue
            q = qTa_s[pl.ds(64 * g + r0, 8), pl.ds(q0, 128)]
            qr = pltpu.roll(q, 64, 1)
            ma = lo & (r8 + r0 >= 9 * ja) & (r8 + r0 < 9 * ja + 9)
            mb = (~lo) & (r8 + r0 >= 9 * jb) & (r8 + r0 < 9 * jb + 9)
            wl.append(jnp.where(ma, q, jnp.where(mb, qr, 0)))
            wu.append(jnp.where(ma, qr, jnp.where(mb, q, 0)))
        return (pltpu.bitcast(jnp.concatenate(wl, axis=0), BF16),
                pltpu.bitcast(jnp.concatenate(wu, axis=0), BF16))

    def a_scores(qt, pr, half, sref, r0, r1, w, mm):
        k0 = pl.multiple_of((qt - 2) * 128 + 64 * half + r0, 64)
        s = jnp.dot(kA_s[(2 * pr) // HA, pl.ds(k0, r1 - r0), :], w, preferred_element_type=F32)
        row = lax.broadcasted_iota(I32, (64, 128), 0)
        key = (row & 48) + 2 * (row & 7) + ((row >> 3) & 1)
        tok = lax.broadcasted_iota(I32, (64, 128), 1) & 63
        for a in range(r0, r1, 64):
            blk = s[a - r0:a - r0 + 64]
            if a < 64:
                blk = jnp.where(key > tok, blk, NEG)
            elif a >= 256:
                blk = jnp.where(key <= tok, blk, NEG)
            sref[a:a + 64, :] = blk
            mm = blk if mm is None else jnp.maximum(mm, blk)
        return mm

    def a_store_max(mm, mref):
        mm = jnp.max(mm.reshape(8, 8, 128), axis=0)
        mref[...] = jnp.broadcast_to(jnp.max(mm, axis=0, keepdims=True), (8, 128))

    def a_probs(sm, r):
        p = jnp.exp2(sm[0][r:r + 64, :] - sm[1][0:1, :]).reshape(4, 2, 8, 128)
        return pltpu.pack_elementwise([p[:, 0], p[:, 1]], packed_dtype=BF16).reshape(32, 128)

    def a_ptiles(sml, smu, t):
        lo = lax.broadcasted_iota(I32, (32, 128), 1) < 64
        pa, pb = [], []
        for r in (128 * t, 128 * t + 64):
            pl_ = a_probs(sml, r) if r < 320 else None
            pu_ = a_probs(smu, r - 64) if r >= 64 else None
            a_lo, b_lo = (pl_, pltpu.roll(pl_, 64, 1)) if pl_ is not None else (0, 0)
            a_hi, b_hi = (pltpu.roll(pu_, 64, 1), pu_) if pu_ is not None else (0, 0)
            pa.append(jnp.where(lo, a_lo, a_hi))
            pb.append(jnp.where(lo, b_lo, b_hi))
        return (pltpu.bitcast(jnp.concatenate(pa, axis=0), BF16),
                pltpu.bitcast(jnp.concatenate(pb, axis=0), BF16))

    def a_pv(qt, h, t, p, acc):
        r24 = lax.broadcasted_iota(I32, (24, 128), 0)
        k0 = pl.multiple_of((qt - 2 + t) * 128, 128)
        r0 = (DH * h) // 8 * 8
        v = jnp.where(r24 == _lrow(h % 4), 1.0, vTa_s[r0:r0 + 24, pl.ds(k0, 128)])
        o = jnp.dot(v, p, preferred_element_type=F32)
        return o if acc is None else acc + o

    def a_all_scores(qt, s, slot, r0, r1, ws, mms):
        return [a_scores(qt, 2 * s + idx // 2, idx % 2, sA_s.at[slot, idx], r0, r1,
                         ws[idx // 2][idx % 2], mms[idx]) for idx in range(4)]

    def a_qtile(qt, oslot, qq):
        for s in range(8):
            slot = s % 2
            if s < 7:
                nqt, ns = qt, s + 1
            else:
                nqt, ns = jnp.minimum(qt + 1, S // 128 - 1), 0
            ws = [a_weights(nqt, 2 * ns + pi) for pi in range(2)]
            accs = [None] * 4

            def pv(t):
                for pi in range(2):
                    pa, pb = a_ptiles(*[(sA_s.at[slot, 2 * pi + hf], mA_s.at[slot, 2 * pi + hf]) for hf in range(2)], t)
                    accs[2 * pi] = a_pv(qt, 4 * s + 2 * pi, t, pa, accs[2 * pi])
                    accs[2 * pi + 1] = a_pv(qt, 4 * s + 2 * pi + 1, t, pb, accs[2 * pi + 1])

            mms = a_all_scores(nqt, ns, 1 - slot, 0, 256, ws, [None] * 4)
            pv(2)
            mms = a_all_scores(nqt, ns, 1 - slot, 256, 320, ws, mms)
            pv(0)
            pv(1)
            for idx in range(4):
                a_store_max(mms[idx], mA_s.at[1 - slot, idx])
            oA_s[oslot, pl.ds(72 * s, 72), pl.ds(qq * 128, 128)] = _assemble(
                [_normalise(accs[hh], hh) for hh in range(4)])

    def out_proj(t):
        rows = pl.ds(pl.multiple_of(t * TF, TF), TF)
        ob = oB_s[:, rows].astype(BF16)
        oa = oA_s[t % 2].astype(BF16)
        for i in range(9):
            if i < 4:
                r = jnp.dot(woT_s[0, 128 * i:128 * (i + 1), :], oa, preferred_element_type=F32)
            elif i == 4:
                ra = jnp.dot(woT_s[0, 512:576, :], oa, preferred_element_type=F32)
                rb = jnp.dot(woT_s[1, 0:64, :], ob, preferred_element_type=F32)
                r = jnp.concatenate([ra, rb], axis=0)
            else:
                r0 = 64 + 128 * (i - 5)
                r = jnp.dot(woT_s[1, r0:r0 + 128, :], ob, preferred_element_type=F32)
            out_s[rows, 128 * i:128 * (i + 1)] = r.astype(BF16).T
            if i == 4:
                out_copy(t, 0).start()
        out_copy(t, 1).start()

    def tile_body(t, carry):
        for qq in range(2):
            a_qtile(2 * t + qq, t % 2, qq)
        out_proj(t - 1)
        return carry

    c_wob.wait()
    c_woa.wait()
    woT_s[0] = wo_s[0].T
    woT_s[1] = wo_s[1].T
    for qt in range(2):
        for pr in range(H // 2):
            ws = a_weights(qt, pr)
            for half in range(2):
                rmin = 256 - 64 * half - 128 * qt
                e = (qt * 16 + pr) * 2 + half
                a_store_max(a_scores(qt, pr, half, sE_s.at[e], rmin, 320, ws[half], None), mE_s.at[e])
    ws = [a_weights(2, pi) for pi in range(2)]
    mm0 = a_all_scores(2, 0, 0, 0, 320, ws, [None] * 4)
    for idx in range(4):
        a_store_max(mm0[idx], mA_s.at[0, idx])
    for qt in range(2):
        for s in range(8):
            accs = [None] * 4
            for t in range(2, 1 - qt, -1):
                for pi in range(2):
                    e = (qt * 16 + 2 * s + pi) * 2
                    pa, pb = a_ptiles((sE_s.at[e], mE_s.at[e]), (sE_s.at[e + 1], mE_s.at[e + 1]), t)
                    accs[2 * pi] = a_pv(qt, 4 * s + 2 * pi, t, pa, accs[2 * pi])
                    accs[2 * pi + 1] = a_pv(qt, 4 * s + 2 * pi + 1, t, pb, accs[2 * pi + 1])
            oA_s[0, pl.ds(72 * s, 72), pl.ds(qt * 128, 128)] = _assemble(
                [_normalise(accs[hh], hh) for hh in range(4)])
    lax.fori_loop(1, NF, tile_body, 0)
    out_proj(NF - 1)
    for t in range(NF):
        out_copy(t, 0).wait()
        out_copy(t, 1).wait()


def _build():
    scratch = [
        pltpu.VMEM((D, S), BF16),
        pltpu.VMEM((D, S), BF16),
        pltpu.VMEM((D, 3 * D), BF16),
        pltpu.VMEM((D, D), BF16),
        pltpu.VMEM((2, D, D), BF16),
        pltpu.VMEM((2, DH, D), BF16),
        pltpu.VMEM((D, D), BF16),
        pltpu.VMEM((3 * D, D), BF16),
        pltpu.VMEM((2, D, D), BF16),
        pltpu.VMEM((48, D), BF16),
        pltpu.VMEM((640, S), BF16),
        pltpu.VMEM((S // 2, 128), I32),
        pltpu.VMEM((4, 24, S), F32),
        pltpu.VMEM((2, S, TQ), F32),
        pltpu.VMEM((8, TQ), F32),
        pltpu.VMEM((3, 24, TQ), F32),
        pltpu.VMEM((D, S + TQ), F32),
        pltpu.VMEM((64 * NGA, S), I32),
        pltpu.VMEM((NGA, S, 128), BF16),

        pltpu.VMEM((D, S), F32),
        pltpu.VMEM((2, 4, 320, 128), F32),
        pltpu.VMEM((2, 4, 8, 128), F32),
        pltpu.VMEM((64, 320, 128), F32),
        pltpu.VMEM((64, 8, 128), F32),
        pltpu.VMEM((2, D, TF), F32),
        pltpu.VMEM((S, 2 * D), BF16),
        pltpu.SemaphoreType.DMA((7,)),
        pltpu.SemaphoreType.DMA((NC,)),
        pltpu.SemaphoreType.DMA((NF, 2)),
    ]
    any_spec = pl.BlockSpec(memory_space=pl.ANY)
    return pl.pallas_call(
        _kernel,
        out_shape=jax.ShapeDtypeStruct((S, 2 * D), BF16),
        in_specs=[any_spec] * 8,
        out_specs=any_spec,
        scratch_shapes=scratch,
        name="concat_heads_window_mqa",
        compiler_params=pltpu.CompilerParams(
            vmem_limit_bytes=100 * 1024 * 1024,
            flags={"XLA_TPU_EVENLY_DISTRIBUTE_CRITICAL_NODES": True},
        ),
    )


@jax.jit
def pallas_concat_heads__sliding_block__grouped_kv_mqa__prompt_kernel(
    A_x: jax.Array,
    A_wqkv: jax.Array,
    A_wo: jax.Array,
    B_x: jax.Array,
    B_wq: jax.Array,
    B_wk: jax.Array,
    B_wv: jax.Array,
    B_wo: jax.Array,
):
    out = _build()(A_x[0].T, A_wqkv, A_wo, B_x[0].T, B_wq, B_wk.T, B_wv.T, B_wo)
    return out.reshape(1, S, 2 * D)
```

```python
import jax
import jax.numpy as jnp
import numpy as np
from jax import lax
from jax.experimental import pallas as pl
from jax.experimental.pallas import tpu as pltpu

S = 2048
D = 576
H = 32
DH = 18
HB = 7
HA = 6
NGA = 6
TQ = 512
NC = S // TQ
KCH = S // 128
NIT = NC * H
UB = 8
TF = 256
NF = S // TF
NEG = -1e30
QSCALE = float(DH ** -0.5 * np.log2(np.e))
F32 = jnp.float32
BF16 = jnp.bfloat16
I32 = jnp.int32


def _pad_group_rows(wt, hpg):
    n = wt.shape[1]
    parts = []
    for lo in range(0, D, hpg * DH):
        hi = min(lo + hpg * DH, D)
        parts.append(wt[lo:hi])
        parts.append(jnp.zeros((128 - (hi - lo), n), wt.dtype))
    return jnp.concatenate(parts, axis=0)


def _lrow(jj):
    return 23 if jj < 3 else 0


def _normalise(o, jj):
    lr = _lrow(jj)
    return o * (1.0 / o[lr:lr + 1, :])


def _assemble(o):
    row8 = lax.broadcasted_iota(I32, (8, o[0].shape[1]), 0)

    def sel(k, a, b):
        return jnp.where(row8 < k, a, b)

    return jnp.concatenate([
        o[0][0:8], o[0][8:16], sel(2, o[0][16:24], o[1][0:8]),
        o[1][8:16], sel(4, o[1][16:24], o[2][0:8]),
        o[2][8:16], sel(6, o[2][16:24], o[3][0:8]),
        o[3][8:16], o[3][16:24]], axis=0)


def _kernel(axT_h, awqkv_h, awo_h, bxT_h, bwq_h, bwkT_h, bwvT_h, bwo_h, out_h,
            xa_s, xb_s, wqkv_s, wq_s, wo_s, wkv_s, wqT_s, wT_s, woT_s, wkvT_s,
            qTb_s, krep_s, vTb_s, sB_s, mB_s, oc_s, oB_s,
            qTa_s, kA_s, vTa_s, sA_s, mA_s, sE_s, mE_s, oA_s, out_s,
            sems, xsems, osems):
    def cp(src, dst, i):
        return pltpu.make_async_copy(src, dst, sems.at[i])

    def xb_copy(c):
        cols = pl.ds(pl.multiple_of(c * TQ, TQ), TQ)
        return pltpu.make_async_copy(bxT_h.at[:, cols], xb_s.at[:, cols], xsems.at[c])

    def out_copy(t, part):
        rows = pl.ds(pl.multiple_of(t * TF, TF), TF)
        cols = pl.ds(0, 640) if part == 0 else pl.ds(640, 512)
        return pltpu.make_async_copy(out_s.at[rows, cols], out_h.at[rows, cols], osems.at[t, part])

    c_wq = cp(bwq_h, wq_s, 0)
    c_wk = cp(bwkT_h, wkv_s.at[0], 1)
    c_wv = cp(bwvT_h, wkv_s.at[1], 2)
    c_wob = cp(bwo_h, wo_s.at[1], 3)
    c_wqkv = cp(awqkv_h, wqkv_s, 4)
    c_xa = cp(axT_h, xa_s, 5)
    c_woa = cp(awo_h, wo_s.at[0], 6)

    c_wk.start()
    c_wv.start()
    c_wq.start()
    sB_s[1] = jnp.zeros((S, TQ), F32)
    mB_s[...] = jnp.zeros((8, TQ), F32)
    oc_s[...] = jnp.zeros((3, 24, TQ), F32)
    c_wk.wait()
    c_wv.wait()
    for c in range(NC):
        xb_copy(c).start()
    c_wqkv.start(priority=1)
    c_xa.start(priority=1)
    c_wob.start(priority=1)
    c_woa.start(priority=1)
    z6 = jnp.zeros((6, D), F32)
    wkvT_s[...] = jnp.concatenate(
        [wkv_s[0].astype(F32), z6, wkv_s[1].astype(F32), z6], axis=0).astype(BF16)
    c_wq.wait()
    wqT_s[...] = wq_s[...].T

    def b_proj(c, carry):
        row24 = lax.broadcasted_iota(I32, (24, TQ), 0)
        cols = pl.ds(pl.multiple_of(c * TQ, TQ), TQ)
        xb_copy(c).wait()
        xT = xb_s[:, cols]
        kvT = jnp.dot(wkvT_s[...], xT, preferred_element_type=F32)
        k = kvT[0:DH]
        kr = jnp.concatenate([k] * 7 + [jnp.zeros((2, TQ), F32)], axis=0).astype(BF16).T
        krep_s[pl.ds(pl.multiple_of(c * (TQ // 2), TQ // 2), TQ // 2), :] = pltpu.bitcast(kr, I32)
        vT = kvT[24:48].astype(BF16).astype(F32)
        for jj in range(4):
            off = 2 * jj
            vv = (jnp.concatenate([jnp.zeros((off, TQ), F32), vT[0:24 - off]], axis=0)
                  if off else vT)
            vTb_s[jj, :, cols] = jnp.where(row24 == _lrow(jj), 1.0, vv)
        qT = jnp.dot(wqT_s[...], xT, preferred_element_type=F32) * QSCALE
        qTb_s[:, cols] = _pad_group_rows(qT, HB).astype(BF16)
        return carry

    lax.fori_loop(0, NC, b_proj, 0)

    def b_kmask(it):
        j = (it % H) % 7
        lane = lax.broadcasted_iota(I32, (8, 128), 1)
        return jnp.where((lane >= DH * j) & (lane < DH * j + DH), I32(-1), I32(0))

    def b_scores(it, c, slot, m, kmask):
        qt = it // H
        g = (it % H) // 7
        w = qTb_s[pl.ds(pl.multiple_of(g * 128, 128), 128), pl.ds(pl.multiple_of(qt * TQ, TQ), TQ)]
        ki = krep_s[pl.ds(c * 64, 64), :].reshape(8, 8, 128) & kmask
        k = pltpu.bitcast(ki.reshape(64, 128), BF16)
        s = jnp.dot(k, w, preferred_element_type=F32)
        sB_s[slot, pl.ds(c * 128, 128), :] = s
        mm = jnp.max(s.reshape(16, 8, TQ), axis=0)
        return mm if m is None else jnp.maximum(m, mm)

    def b_pv(c, slot, jj, m, acc):
        p = jnp.exp2(sB_s[slot, pl.ds(c * 128, 128), :] - m).astype(BF16)
        o = jnp.dot(vTb_s[jj, :, pl.ds(c * 128, 128)], p, preferred_element_type=F32)
        return o if acc is None else acc + o

    def b_store_unit(iu, outs):
        oB_s[pl.ds(pl.multiple_of((iu % 8) * 72, 8), 72),
             pl.ds(pl.multiple_of((iu // 8) * TQ, TQ), TQ)] = _assemble(outs)

    def b_body(i, carry):
        seq = [(st, c) for st in range(UB) for c in range(KCH)]
        mx, ms, accs, kmasks, outs = {}, {}, {}, {}, {}
        for n in range(len(seq) + 1):
            if n < len(seq):
                st, c = seq[n]
                it = i * UB + st
                if c == 0:
                    kmasks[st] = b_kmask(it)
                mx[st] = b_scores(it, c, st % 2, mx.get(st), kmasks[st])
            if n >= 1:
                st, c = seq[n - 1]
                jj = (st - 1) % 4
                if c == 0:
                    ms[st] = (mB_s[...][0:1, :] if st == 0
                              else jnp.max(mx[st - 1], axis=0, keepdims=True))
                accs[st] = b_pv(c, (st - 1) % 2, jj, ms[st], accs.get(st))
                if c == KCH - 1:
                    outs[jj] = _normalise(accs[st], jj)
                    if st == 0:
                        iu = jnp.where(i == 0, NIT // 4, i * (UB // 4) - 1)
                        b_store_unit(iu, [oc_s[0], oc_s[1], oc_s[2], outs[3]])
                    elif jj == 3:
                        b_store_unit(i * (UB // 4) + st // 4 - 1, outs)
        for jj in range(3):
            oc_s[jj] = outs[jj]
        mB_s[...] = jnp.broadcast_to(jnp.max(mx[UB - 1], axis=0, keepdims=True), (8, TQ))
        return carry

    lax.fori_loop(0, NIT // UB, b_body, 0)

    def a_cols(c):
        return pl.ds(pl.multiple_of(c * TQ, TQ), TQ)

    def a_proj_k(c):
        cols = a_cols(c)
        kT = jnp.dot(wT_s[D:2 * D, :], xa_s[:, cols], preferred_element_type=F32)
        kT = _pad_group_rows(kT, HA)
        for g in range(NGA):
            n = pltpu.bitcast(kT[128 * g:128 * (g + 1)].astype(BF16).T, I32).reshape(TQ // 16, 1, 8, 128)
            even = lax.bitcast_convert_type(n << 16, F32)
            odd = lax.bitcast_convert_type(n & I32(-65536), F32)
            kA_s[g, cols, :] = jnp.concatenate([even, odd], axis=1).reshape(TQ, 128).astype(BF16)

    def a_proj_q(c):
        cols = a_cols(c)
        qT = jnp.dot(wT_s[0:D, :], xa_s[:, cols], preferred_element_type=F32) * QSCALE
        qTa_s[:, cols] = pltpu.bitcast(_pad_group_rows(qT, HA).astype(BF16), I32)

    def a_proj_v(c):
        cols = a_cols(c)
        vT = jnp.dot(wT_s[2 * D:3 * D, :], xa_s[:, cols], preferred_element_type=F32)
        vTa_s[:, cols] = vT.astype(BF16).astype(F32)

    def a_proj(c, carry):
        a_proj_k(c)
        a_proj_q(c)
        a_proj_v(c)
        return carry

    c_wqkv.wait()
    c_xa.wait()
    m_last = mB_s[...][0:1, :]
    acc = None
    wT_s[2 * D:3 * D, :] = wqkv_s[:, 2 * D:3 * D].T
    a_proj_v(0)
    for c in range(0, 5):
        acc = b_pv(c, 1, 3, m_last, acc)
    wT_s[0:640, :] = wqkv_s[:, 0:640].T
    a_proj_q(0)
    for c in range(5, 11):
        acc = b_pv(c, 1, 3, m_last, acc)
    wT_s[640:2 * D, :] = wqkv_s[:, 640:2 * D].T
    a_proj_k(0)
    for c in range(11, KCH):
        acc = b_pv(c, 1, 3, m_last, acc)
    b_store_unit(NIT // 4 - 1, [oc_s[0], oc_s[1], oc_s[2], _normalise(acc, 3)])
    lax.fori_loop(1, NC, a_proj, 0)

    def a_weights(qt, pr):
        g, ja = (2 * pr) // HA, (2 * pr) % HA
        jb = ja + 1
        q0 = pl.multiple_of(qt * 128, 128)
        r8 = lax.broadcasted_iota(I32, (8, 128), 0)
        lo = lax.broadcasted_iota(I32, (8, 128), 1) < 64
        wl, wu = [], []
        for r0 in range(0, 64, 8):
            if r0 + 8 <= 9 * ja or r0 >= 9 * jb + 9:
                wl.append(jnp.zeros((8, 128), I32))
                wu.append(jnp.zeros((8, 128), I32))
                continue
            q = qTa_s[pl.ds(64 * g + r0, 8), pl.ds(q0, 128)]
            qr = pltpu.roll(q, 64, 1)
            ma = lo & (r8 + r0 >= 9 * ja) & (r8 + r0 < 9 * ja + 9)
            mb = (~lo) & (r8 + r0 >= 9 * jb) & (r8 + r0 < 9 * jb + 9)
            wl.append(jnp.where(ma, q, jnp.where(mb, qr, 0)))
            wu.append(jnp.where(ma, qr, jnp.where(mb, q, 0)))
        return (pltpu.bitcast(jnp.concatenate(wl, axis=0), BF16),
                pltpu.bitcast(jnp.concatenate(wu, axis=0), BF16))

    def a_scores(qt, pr, half, sref, r0, r1, w, mm):
        k0 = pl.multiple_of((qt - 2) * 128 + 64 * half + r0, 64)
        s = jnp.dot(kA_s[(2 * pr) // HA, pl.ds(k0, r1 - r0), :], w, preferred_element_type=F32)
        row = lax.broadcasted_iota(I32, (64, 128), 0)
        key = (row & 48) + 2 * (row & 7) + ((row >> 3) & 1)
        tok = lax.broadcasted_iota(I32, (64, 128), 1) & 63
        for a in range(r0, r1, 64):
            blk = s[a - r0:a - r0 + 64]
            if a < 64:
                blk = jnp.where(key > tok, blk, NEG)
            elif a >= 256:
                blk = jnp.where(key <= tok, blk, NEG)
            sref[a:a + 64, :] = blk
            mm = blk if mm is None else jnp.maximum(mm, blk)
        return mm

    def a_store_max(mm, mref):
        mm = jnp.max(mm.reshape(8, 8, 128), axis=0)
        mref[...] = jnp.broadcast_to(jnp.max(mm, axis=0, keepdims=True), (8, 128))

    def a_probs(sm, r):
        p = jnp.exp2(sm[0][r:r + 64, :] - sm[1][0:1, :]).reshape(4, 2, 8, 128)
        u = lax.bitcast_convert_type(p, I32)
        return (lax.shift_right_logical(u[:, 0], 16) | (u[:, 1] & I32(-65536))).reshape(32, 128)

    def a_ptiles(sml, smu, t):
        lo = lax.broadcasted_iota(I32, (32, 128), 1) < 64
        pa, pb = [], []
        for r in (128 * t, 128 * t + 64):
            pl_ = a_probs(sml, r) if r < 320 else None
            pu_ = a_probs(smu, r - 64) if r >= 64 else None
            a_lo, b_lo = (pl_, pltpu.roll(pl_, 64, 1)) if pl_ is not None else (0, 0)
            a_hi, b_hi = (pltpu.roll(pu_, 64, 1), pu_) if pu_ is not None else (0, 0)
            pa.append(jnp.where(lo, a_lo, a_hi))
            pb.append(jnp.where(lo, b_lo, b_hi))
        return (pltpu.bitcast(jnp.concatenate(pa, axis=0), BF16),
                pltpu.bitcast(jnp.concatenate(pb, axis=0), BF16))

    def a_pv(qt, h, t, p, acc):
        r24 = lax.broadcasted_iota(I32, (24, 128), 0)
        k0 = pl.multiple_of((qt - 2 + t) * 128, 128)
        r0 = (DH * h) // 8 * 8
        v = jnp.where(r24 == _lrow(h % 4), 1.0, vTa_s[r0:r0 + 24, pl.ds(k0, 128)])
        o = jnp.dot(v, p, preferred_element_type=F32)
        return o if acc is None else acc + o

    def a_all_scores(qt, s, slot, r0, r1, ws, mms):
        return [a_scores(qt, 2 * s + idx // 2, idx % 2, sA_s.at[slot, idx], r0, r1,
                         ws[idx // 2][idx % 2], mms[idx]) for idx in range(4)]

    def a_qtile(qt, oslot, qq):
        for s in range(8):
            slot = s % 2
            if s < 7:
                nqt, ns = qt, s + 1
            else:
                nqt, ns = jnp.minimum(qt + 1, S // 128 - 1), 0
            ws = [a_weights(nqt, 2 * ns + pi) for pi in range(2)]
            accs = [None] * 4

            def pv(t):
                for pi in range(2):
                    pa, pb = a_ptiles(*[(sA_s.at[slot, 2 * pi + hf], mA_s.at[slot, 2 * pi + hf])
                                        for hf in range(2)], t)
                    accs[2 * pi] = a_pv(qt, 4 * s + 2 * pi, t, pa, accs[2 * pi])
                    accs[2 * pi + 1] = a_pv(qt, 4 * s + 2 * pi + 1, t, pb, accs[2 * pi + 1])

            mms = a_all_scores(nqt, ns, 1 - slot, 0, 256, ws, [None] * 4)
            pv(2)
            mms = a_all_scores(nqt, ns, 1 - slot, 256, 320, ws, mms)
            pv(0)
            pv(1)
            for idx in range(4):
                a_store_max(mms[idx], mA_s.at[1 - slot, idx])
            oA_s[oslot, pl.ds(72 * s, 72), pl.ds(qq * 128, 128)] = _assemble(
                [_normalise(accs[hh], hh) for hh in range(4)])

    def out_proj(t):
        rows = pl.ds(pl.multiple_of(t * TF, TF), TF)
        ob = oB_s[:, rows].astype(BF16)
        oa = oA_s[t % 2].astype(BF16)
        for i in range(9):
            if i < 4:
                r = jnp.dot(woT_s[0, 128 * i:128 * (i + 1), :], oa, preferred_element_type=F32)
            elif i == 4:
                ra = jnp.dot(woT_s[0, 512:576, :], oa, preferred_element_type=F32)
                rb = jnp.dot(woT_s[1, 0:64, :], ob, preferred_element_type=F32)
                r = jnp.concatenate([ra, rb], axis=0)
            else:
                r0 = 64 + 128 * (i - 5)
                r = jnp.dot(woT_s[1, r0:r0 + 128, :], ob, preferred_element_type=F32)
            out_s[rows, 128 * i:128 * (i + 1)] = r.astype(BF16).T
            if i == 4:
                out_copy(t, 0).start()
        out_copy(t, 1).start()

    def tile_body(t, carry):
        for qq in range(2):
            a_qtile(2 * t + qq, t % 2, qq)
        out_proj(t - 1)
        return carry

    c_wob.wait()
    c_woa.wait()
    woT_s[0] = wo_s[0].T
    woT_s[1] = wo_s[1].T
    for qt in range(2):
        for pr in range(H // 2):
            ws = a_weights(qt, pr)
            for half in range(2):
                rmin = 256 - 64 * half - 128 * qt
                e = (qt * 16 + pr) * 2 + half
                a_store_max(a_scores(qt, pr, half, sE_s.at[e], rmin, 320, ws[half], None), mE_s.at[e])
    ws = [a_weights(2, pi) for pi in range(2)]
    mm0 = a_all_scores(2, 0, 0, 0, 320, ws, [None] * 4)
    for idx in range(4):
        a_store_max(mm0[idx], mA_s.at[0, idx])
    for qt in range(2):
        for s in range(8):
            accs = [None] * 4
            for t in range(2, 1 - qt, -1):
                for pi in range(2):
                    e = (qt * 16 + 2 * s + pi) * 2
                    pa, pb = a_ptiles((sE_s.at[e], mE_s.at[e]), (sE_s.at[e + 1], mE_s.at[e + 1]), t)
                    accs[2 * pi] = a_pv(qt, 4 * s + 2 * pi, t, pa, accs[2 * pi])
                    accs[2 * pi + 1] = a_pv(qt, 4 * s + 2 * pi + 1, t, pb, accs[2 * pi + 1])
            oA_s[0, pl.ds(72 * s, 72), pl.ds(qt * 128, 128)] = _assemble(
                [_normalise(accs[hh], hh) for hh in range(4)])
    lax.fori_loop(1, NF, tile_body, 0)
    out_proj(NF - 1)
    for t in range(NF):
        out_copy(t, 0).wait()
        out_copy(t, 1).wait()


def _build():
    scratch = [
        pltpu.VMEM((D, S), BF16),
        pltpu.VMEM((D, S), BF16),
        pltpu.VMEM((D, 3 * D), BF16),
        pltpu.VMEM((D, D), BF16),
        pltpu.VMEM((2, D, D), BF16),
        pltpu.VMEM((2, DH, D), BF16),
        pltpu.VMEM((D, D), BF16),
        pltpu.VMEM((3 * D, D), BF16),
        pltpu.VMEM((2, D, D), BF16),
        pltpu.VMEM((48, D), BF16),
        pltpu.VMEM((640, S), BF16),
        pltpu.VMEM((S // 2, 128), I32),
        pltpu.VMEM((4, 24, S), F32),
        pltpu.VMEM((2, S, TQ), F32),
        pltpu.VMEM((8, TQ), F32),
        pltpu.VMEM((3, 24, TQ), F32),
        pltpu.VMEM((D, S + TQ), F32),
        pltpu.VMEM((64 * NGA, S), I32),
        pltpu.VMEM((NGA, S, 128), BF16),

        pltpu.VMEM((D, S), F32),
        pltpu.VMEM((2, 4, 320, 128), F32),
        pltpu.VMEM((2, 4, 8, 128), F32),
        pltpu.VMEM((64, 320, 128), F32),
        pltpu.VMEM((64, 8, 128), F32),
        pltpu.VMEM((2, D, TF), F32),
        pltpu.VMEM((S, 2 * D), BF16),
        pltpu.SemaphoreType.DMA((7,)),
        pltpu.SemaphoreType.DMA((NC,)),
        pltpu.SemaphoreType.DMA((NF, 2)),
    ]
    any_spec = pl.BlockSpec(memory_space=pl.ANY)
    return pl.pallas_call(
        _kernel,
        out_shape=jax.ShapeDtypeStruct((S, 2 * D), BF16),
        in_specs=[any_spec] * 8,
        out_specs=any_spec,
        scratch_shapes=scratch,
        name="concat_heads_window_mqa",
        compiler_params=pltpu.CompilerParams(
            vmem_limit_bytes=100 * 1024 * 1024,
            flags={"XLA_TPU_EVENLY_DISTRIBUTE_CRITICAL_NODES": True},
        ),
    )


@jax.jit
def pallas_concat_heads__sliding_block__grouped_kv_mqa__prompt_kernel(
    A_x: jax.Array,
    A_wqkv: jax.Array,
    A_wo: jax.Array,
    B_x: jax.Array,
    B_wq: jax.Array,
    B_wk: jax.Array,
    B_wv: jax.Array,
    B_wo: jax.Array,
):
    out = _build()(A_x[0].T, A_wqkv, A_wo, B_x[0].T, B_wq, B_wk.T, B_wv.T, B_wo)
    return out.reshape(1, S, 2 * D)
```

```python
import jax
import jax.numpy as jnp
import numpy as np
from jax import lax
from jax.experimental import pallas as pl
from jax.experimental.pallas import tpu as pltpu

S = 2048
D = 576
H = 32
DH = 18
NG = 5
TQ = 512
NC = S // TQ
KCH = S // 128
NIT = NC * H
UB = 8
TF = 256
NF = S // TF
NEG = -1e30
QSCALE = float(DH ** -0.5 * np.log2(np.e))
F32 = jnp.float32
BF16 = jnp.bfloat16
I32 = jnp.int32


def _pad_group_rows(wt):
    n = wt.shape[1]
    parts = []
    for g in range(NG):
        lo = 126 * g
        hi = min(lo + 126, D)
        parts.append(wt[lo:hi])
        parts.append(jnp.zeros((128 - (hi - lo), n), wt.dtype))
    return jnp.concatenate(parts, axis=0)


def _lrow(jj):
    return 23 if jj < 3 else 0


def _normalise(o, jj):
    lr = _lrow(jj)
    return o * (1.0 / o[lr:lr + 1, :])


def _assemble(o):
    row8 = lax.broadcasted_iota(I32, (8, o[0].shape[1]), 0)

    def sel(k, a, b):
        return jnp.where(row8 < k, a, b)

    return jnp.concatenate([
        o[0][0:8], o[0][8:16], sel(2, o[0][16:24], o[1][0:8]),
        o[1][8:16], sel(4, o[1][16:24], o[2][0:8]),
        o[2][8:16], sel(6, o[2][16:24], o[3][0:8]),
        o[3][8:16], o[3][16:24]], axis=0)


def _kernel(axT_h, awqkv_h, awo_h, bxT_h, bwq_h, bwkT_h, bwvT_h, bwo_h, out_h,
            xa_s, xb_s, wqkv_s, wq_s, wo_s, wkv_s, wqT_s, wT_s, woT_s, wkvT_s,
            qTb_s, krep_s, vTb_s, sB_s, mB_s, oc_s, oB_s,
            qTa_s, kA_s, vTa_s, sA_s, mA_s, oA_s, out_s,
            sems, xsems, osems):
    def cp(src, dst, i):
        return pltpu.make_async_copy(src, dst, sems.at[i])

    def xb_copy(c):
        cols = pl.ds(pl.multiple_of(c * TQ, TQ), TQ)
        return pltpu.make_async_copy(bxT_h.at[:, cols], xb_s.at[:, cols], xsems.at[c])

    def out_copy(t, part):
        rows = pl.ds(pl.multiple_of(t * TF, TF), TF)
        cols = pl.ds(0, 640) if part == 0 else pl.ds(640, 512)
        return pltpu.make_async_copy(out_s.at[rows, cols], out_h.at[rows, cols], osems.at[t, part])

    c_wq = cp(bwq_h, wq_s, 0)
    c_wk = cp(bwkT_h, wkv_s.at[0], 1)
    c_wv = cp(bwvT_h, wkv_s.at[1], 2)
    c_wob = cp(bwo_h, wo_s.at[1], 3)
    c_wqkv = cp(awqkv_h, wqkv_s, 4)
    c_xa = cp(axT_h, xa_s, 5)
    c_woa = cp(awo_h, wo_s.at[0], 6)

    c_wk.start()
    c_wv.start()
    c_wq.start()
    sB_s[1] = jnp.zeros((S, TQ), F32)
    mB_s[...] = jnp.zeros((8, TQ), F32)
    oc_s[...] = jnp.zeros((3, 24, TQ), F32)
    c_wk.wait()
    c_wv.wait()
    for c in range(NC):
        xb_copy(c).start()
    c_wqkv.start(priority=1)
    c_xa.start(priority=1)
    c_wob.start(priority=1)
    c_woa.start(priority=1)
    z6 = jnp.zeros((6, D), F32)
    wkvT_s[...] = jnp.concatenate(
        [wkv_s[0].astype(F32), z6, wkv_s[1].astype(F32), z6], axis=0).astype(BF16)
    c_wq.wait()
    wqT_s[...] = wq_s[...].T

    def b_proj(c, carry):
        row24 = lax.broadcasted_iota(I32, (24, TQ), 0)
        cols = pl.ds(pl.multiple_of(c * TQ, TQ), TQ)
        xb_copy(c).wait()
        xT = xb_s[:, cols]
        kvT = jnp.dot(wkvT_s[...], xT, preferred_element_type=F32)
        k = kvT[0:DH]
        kr = jnp.concatenate([k] * 7 + [jnp.zeros((2, TQ), F32)], axis=0).astype(BF16).T
        krep_s[pl.ds(pl.multiple_of(c * (TQ // 2), TQ // 2), TQ // 2), :] = pltpu.bitcast(kr, I32)
        vT = kvT[24:48].astype(BF16).astype(F32)
        for jj in range(4):
            off = 2 * jj
            vv = (jnp.concatenate([jnp.zeros((off, TQ), F32), vT[0:24 - off]], axis=0)
                  if off else vT)
            vTb_s[jj, :, cols] = jnp.where(row24 == _lrow(jj), 1.0, vv)
        qT = jnp.dot(wqT_s[...], xT, preferred_element_type=F32) * QSCALE
        qTb_s[:, cols] = _pad_group_rows(qT).astype(BF16)
        return carry

    lax.fori_loop(0, NC, b_proj, 0)

    def b_kmask(it):
        j = (it % H) % 7
        lane = lax.broadcasted_iota(I32, (8, 128), 1)
        return jnp.where((lane >= DH * j) & (lane < DH * j + DH), I32(-1), I32(0))

    def b_scores(it, c, slot, m, kmask):
        qt = it // H
        g = (it % H) // 7
        w = qTb_s[pl.ds(pl.multiple_of(g * 128, 128), 128), pl.ds(pl.multiple_of(qt * TQ, TQ), TQ)]
        ki = krep_s[pl.ds(c * 64, 64), :].reshape(8, 8, 128) & kmask
        k = pltpu.bitcast(ki.reshape(64, 128), BF16)
        s = jnp.dot(k, w, preferred_element_type=F32)
        sB_s[slot, pl.ds(c * 128, 128), :] = s
        mm = jnp.max(s.reshape(16, 8, TQ), axis=0)
        return mm if m is None else jnp.maximum(m, mm)

    def b_pv(c, slot, jj, m, acc):
        p = jnp.exp2(sB_s[slot, pl.ds(c * 128, 128), :] - m).astype(BF16)
        o = jnp.dot(vTb_s[jj, :, pl.ds(c * 128, 128)], p, preferred_element_type=F32)
        return o if acc is None else acc + o

    def b_store_unit(iu, outs):
        oB_s[pl.ds(pl.multiple_of((iu % 8) * 72, 8), 72),
             pl.ds(pl.multiple_of((iu // 8) * TQ, TQ), TQ)] = _assemble(outs)

    def b_body(i, carry):
        seq = [(st, c) for st in range(UB) for c in range(KCH)]
        mx, ms, accs, kmasks, outs = {}, {}, {}, {}, {}
        for n in range(len(seq) + 1):
            if n < len(seq):
                st, c = seq[n]
                it = i * UB + st
                if c == 0:
                    kmasks[st] = b_kmask(it)
                mx[st] = b_scores(it, c, st % 2, mx.get(st), kmasks[st])
            if n >= 1:
                st, c = seq[n - 1]
                jj = (st - 1) % 4
                if c == 0:
                    ms[st] = (mB_s[...][0:1, :] if st == 0
                              else jnp.max(mx[st - 1], axis=0, keepdims=True))
                accs[st] = b_pv(c, (st - 1) % 2, jj, ms[st], accs.get(st))
                if c == KCH - 1:
                    outs[jj] = _normalise(accs[st], jj)
                    if st == 0:
                        iu = jnp.where(i == 0, NIT // 4, i * (UB // 4) - 1)
                        b_store_unit(iu, [oc_s[0], oc_s[1], oc_s[2], outs[3]])
                    elif jj == 3:
                        b_store_unit(i * (UB // 4) + st // 4 - 1, outs)
        for jj in range(3):
            oc_s[jj] = outs[jj]
        mB_s[...] = jnp.broadcast_to(jnp.max(mx[UB - 1], axis=0, keepdims=True), (8, TQ))
        return carry

    lax.fori_loop(0, NIT // UB, b_body, 0)

    def a_cols(c):
        return pl.ds(pl.multiple_of(c * TQ, TQ), TQ)

    def a_proj_k(c):
        cols = a_cols(c)
        kT = jnp.dot(wT_s[D:2 * D, :], xa_s[:, cols], preferred_element_type=F32)
        kT = _pad_group_rows(kT).astype(BF16)
        for g in range(NG):
            kA_s[g, cols, :] = kT[128 * g:128 * (g + 1)].T

    def a_proj_q(c):
        cols = a_cols(c)
        qT = jnp.dot(wT_s[0:D, :], xa_s[:, cols], preferred_element_type=F32) * QSCALE
        qTa_s[:, cols] = pltpu.bitcast(_pad_group_rows(qT).astype(BF16), I32)

    def a_proj_v(c):
        cols = a_cols(c)
        vT = jnp.dot(wT_s[2 * D:3 * D, :], xa_s[:, cols], preferred_element_type=F32)
        vTa_s[:, cols] = vT.astype(BF16).astype(F32)

    def a_proj(c, carry):
        a_proj_k(c)
        a_proj_q(c)
        a_proj_v(c)
        return carry

    c_wqkv.wait()
    c_xa.wait()
    m_last = mB_s[...][0:1, :]
    acc = None
    wT_s[2 * D:3 * D, :] = wqkv_s[:, 2 * D:3 * D].T
    a_proj_v(0)
    for c in range(0, 5):
        acc = b_pv(c, 1, 3, m_last, acc)
    wT_s[0:640, :] = wqkv_s[:, 0:640].T
    a_proj_q(0)
    for c in range(5, 11):
        acc = b_pv(c, 1, 3, m_last, acc)
    wT_s[640:2 * D, :] = wqkv_s[:, 640:2 * D].T
    a_proj_k(0)
    for c in range(11, KCH):
        acc = b_pv(c, 1, 3, m_last, acc)
    b_store_unit(NIT // 4 - 1, [oc_s[0], oc_s[1], oc_s[2], _normalise(acc, 3)])
    lax.fori_loop(1, NC, a_proj, 0)

    def a_weights(qt, h):
        r8 = lax.broadcasted_iota(I32, (8, 128), 0)
        g, j = h // 7, h % 7
        q0 = pl.multiple_of(qt * 128, 128)
        lo, hi = 9 * j, 9 * j + 9
        blocks = []
        for b in range(8):
            r0 = 8 * b
            if r0 + 8 <= lo or r0 >= hi:
                blk = jnp.zeros((8, 128), I32)
            else:
                blk = qTa_s[pl.ds(64 * g + r0, 8), pl.ds(q0, 128)]
                if not (r0 >= lo and r0 + 8 <= hi):
                    blk = jnp.where((r8 + r0 >= lo) & (r8 + r0 < hi), blk, I32(0))
            blocks.append(blk)
        return pltpu.bitcast(jnp.concatenate(blocks, axis=0), BF16)

    def a_scores(qt, h, slot, hh, r0, r1, w, mm):
        k0 = pl.multiple_of((qt - 2) * 128 + r0, 64)
        s = jnp.dot(kA_s[h // 7, pl.ds(k0, r1 - r0), :], w, preferred_element_type=F32)
        r64 = lax.broadcasted_iota(I32, (64, 128), 0)
        l64 = lax.broadcasted_iota(I32, (64, 128), 1)
        for a in range(r0, r1, 64):
            blk = s[a - r0:a - r0 + 64]
            if a < 128:
                blk = jnp.where(r64 + a > l64, blk, NEG)
            elif a >= 256:
                blk = jnp.where(r64 + (a - 256) <= l64, blk, NEG)
            sA_s[slot, hh, a:a + 64, :] = blk
            mm = blk if mm is None else jnp.maximum(mm, blk)
        return mm

    def a_store_max(mm, slot, hh):
        mm = jnp.max(mm.reshape(8, 8, 128), axis=0)
        mA_s[slot, hh] = jnp.broadcast_to(jnp.max(mm, axis=0, keepdims=True), (8, 128))

    def a_pv(qt, h, slot, hh, t, acc):
        r24 = lax.broadcasted_iota(I32, (24, 128), 0)
        k0 = pl.multiple_of((qt - 2 + t) * 128, 128)
        r0 = (DH * h) // 8 * 8
        m = mA_s[slot, hh][0:1, :]
        p = jnp.exp2(sA_s[slot, hh, 128 * t:128 * (t + 1), :] - m).astype(BF16)
        v = jnp.where(r24 == _lrow(h % 4), 1.0, vTa_s[r0:r0 + 24, pl.ds(k0, 128)])
        o = jnp.dot(v, p, preferred_element_type=F32)
        return o if acc is None else acc + o

    def a_qtile(qt, oslot, qq, tmin=0, tmin_next=0):
        for s in range(8):
            slot = s % 2
            if s < 7:
                nqt, nh0, nmin = qt, (s + 1) * 4, tmin
            else:
                nqt, nh0, nmin = jnp.minimum(qt + 1, S // 128 - 1), 0, tmin_next
            hs = range(4)
            ws = [a_weights(nqt, nh0 + hh) for hh in hs]
            accs = [None] * 4
            mms = [None] * 4
            if nmin < 2:
                mms = [a_scores(nqt, nh0 + hh, 1 - slot, hh, 128 * nmin, 256, ws[hh], None)
                       for hh in hs]
            if tmin == 0:
                accs = [a_pv(qt, s * 4 + hh, slot, hh, 0, None) for hh in hs]
            mms = [a_scores(nqt, nh0 + hh, 1 - slot, hh, 256, 384, ws[hh], mms[hh]) for hh in hs]
            for t in range(max(tmin, 1), 3):
                accs = [a_pv(qt, s * 4 + hh, slot, hh, t, accs[hh]) for hh in hs]
            for hh in hs:
                a_store_max(mms[hh], 1 - slot, hh)
            oA_s[oslot, pl.ds(72 * s, 72), pl.ds(qq * 128, 128)] = _assemble(
                [_normalise(accs[hh], hh) for hh in hs])

    def attn_tile(t):
        for qq in range(2):
            a_qtile(2 * t + qq, t % 2, qq)

    def out_proj(t):
        rows = pl.ds(pl.multiple_of(t * TF, TF), TF)
        ob = oB_s[:, rows].astype(BF16)
        oa = oA_s[t % 2].astype(BF16)
        for i in range(9):
            if i < 4:
                r = jnp.dot(woT_s[0, 128 * i:128 * (i + 1), :], oa, preferred_element_type=F32)
            elif i == 4:
                ra = jnp.dot(woT_s[0, 512:576, :], oa, preferred_element_type=F32)
                rb = jnp.dot(woT_s[1, 0:64, :], ob, preferred_element_type=F32)
                r = jnp.concatenate([ra, rb], axis=0)
            else:
                r0 = 64 + 128 * (i - 5)
                r = jnp.dot(woT_s[1, r0:r0 + 128, :], ob, preferred_element_type=F32)
            out_s[rows, 128 * i:128 * (i + 1)] = r.astype(BF16).T
            if i == 4:
                out_copy(t, 0).start()
        out_copy(t, 1).start()

    def tile_body(t, carry):
        out_proj(t - 1)
        attn_tile(t)
        return carry

    c_wob.wait()
    c_woa.wait()
    woT_s[0] = wo_s[0].T
    woT_s[1] = wo_s[1].T
    for hh in range(4):
        a_store_max(a_scores(0, hh, 0, hh, 256, 384, a_weights(0, hh), None), 0, hh)
    a_qtile(0, 0, 0, tmin=2, tmin_next=1)
    a_qtile(1, 0, 1, tmin=1, tmin_next=0)
    lax.fori_loop(1, NF, tile_body, 0)
    out_proj(NF - 1)
    for t in range(NF):
        out_copy(t, 0).wait()
        out_copy(t, 1).wait()


def _build():
    scratch = [
        pltpu.VMEM((D, S), BF16),
        pltpu.VMEM((D, S), BF16),
        pltpu.VMEM((D, 3 * D), BF16),
        pltpu.VMEM((D, D), BF16),
        pltpu.VMEM((2, D, D), BF16),
        pltpu.VMEM((2, DH, D), BF16),
        pltpu.VMEM((D, D), BF16),
        pltpu.VMEM((3 * D, D), BF16),
        pltpu.VMEM((2, D, D), BF16),
        pltpu.VMEM((48, D), BF16),
        pltpu.VMEM((640, S), BF16),
        pltpu.VMEM((S // 2, 128), I32),
        pltpu.VMEM((4, 24, S), F32),
        pltpu.VMEM((2, S, TQ), F32),
        pltpu.VMEM((8, TQ), F32),
        pltpu.VMEM((3, 24, TQ), F32),
        pltpu.VMEM((D, S + TQ), F32),
        pltpu.VMEM((320, S), I32),
        pltpu.VMEM((NG, S, 128), BF16),
        pltpu.VMEM((D, S), F32),
        pltpu.VMEM((2, 4, 384, 128), F32),
        pltpu.VMEM((2, 4, 8, 128), F32),
        pltpu.VMEM((2, D, TF), F32),
        pltpu.VMEM((S, 2 * D), BF16),
        pltpu.SemaphoreType.DMA((7,)),
        pltpu.SemaphoreType.DMA((NC,)),
        pltpu.SemaphoreType.DMA((NF, 2)),
    ]
    any_spec = pl.BlockSpec(memory_space=pl.ANY)
    return pl.pallas_call(
        _kernel,
        out_shape=jax.ShapeDtypeStruct((S, 2 * D), BF16),
        in_specs=[any_spec] * 8,
        out_specs=any_spec,
        scratch_shapes=scratch,
        name="concat_heads_window_mqa",
        compiler_params=pltpu.CompilerParams(
            vmem_limit_bytes=100 * 1024 * 1024,
            flags={"XLA_TPU_EVENLY_DISTRIBUTE_CRITICAL_NODES": True},
        ),
    )


@jax.jit
def pallas_concat_heads__sliding_block__grouped_kv_mqa__prompt_kernel(
    A_x: jax.Array,
    A_wqkv: jax.Array,
    A_wo: jax.Array,
    B_x: jax.Array,
    B_wq: jax.Array,
    B_wk: jax.Array,
    B_wv: jax.Array,
    B_wo: jax.Array,
):
    out = _build()(A_x[0].T, A_wqkv, A_wo, B_x[0].T, B_wq, B_wk.T, B_wv.T, B_wo)
    return out.reshape(1, S, 2 * D)
```
